```python
import jax
import jax.numpy as jnp

def _softmax(x, axis=-1):
    return jax.nn.softmax(x, axis=axis)
def _gelu(x):
    return jax.nn.gelu(x, approximate=True)
def _silu(x):
    return jax.nn.silu(x)
def _sigmoid(x):
    return jax.nn.sigmoid(x)
def _layernorm(x, axis=-1, eps=1e-5):
    m = jnp.mean(x, axis=axis, keepdims=True)
    v = jnp.var(x, axis=axis, keepdims=True)
    return (x - m) / jnp.sqrt(v + eps)
def _scatter_add(tgt, idx, src, axis=0):
    return tgt.at[idx].add(src)
def _segment_sum(src, seg, n):
    return jax.ops.segment_sum(src, seg, n)
class _Rng:
    def __init__(self, key):
        self._k = key
    def _next(self):
        self._k, sub = jax.random.split(self._k)
        return sub
    def normal(self, shape):
        return jax.random.normal(self._next(), shape, dtype=jnp.bfloat16)
    def randint(self, lo, hi, shape):
        return jax.random.randint(self._next(), shape, lo, hi, dtype=jnp.int32)
    def uniform(self, shape, lo=0.0, hi=1.0):
        return jax.random.uniform(self._next(), shape, jnp.bfloat16, lo, hi)
    def permutation(self, n):
        return jax.random.permutation(self._next(), n)


kernel_name = 'parallel_sum__linear_kernel_hedgehog__glu_gated_geglu__prompt'

def _fwd_setup_inputs():
    _rng = _Rng(jax.random.key(int.from_bytes(__import__("os").urandom(4), "little")))
    _w = (lambda a: (lambda t: t.astype(jnp.bfloat16) if jnp.issubdtype(t.dtype, jnp.floating) else t)(jnp.asarray(a)))
    def _A_setup():
        B, S, D, H = 1, 2048, 448, 16
        Dh = D // H
        return {
            "x": _w((lambda *s: _rng.normal(s) * 0.05)(B, S, D)),
            "wqkv": _w((lambda *s: _rng.normal(s) * 0.05)(D, 3 * D)),
            "w_phi": _w((lambda *s: _rng.normal(s) * 0.05)(H, Dh, Dh) * (Dh ** -0.5)),
            "wo": _w((lambda *s: _rng.normal(s) * 0.05)(D, D)),
        }
    _A_in = _A_setup()

    def _B_setup():
        B, S, Dm, Df = 1, 2048, 448, 1792
        return {
            "x": _w((lambda *s: _rng.normal(s) * 0.05)(B, S, Dm)),
            "w_gate": _w((lambda *s: _rng.normal(s) * 0.05)(Dm, Df) * (Dm ** -0.5)),
            "w_up": _w((lambda *s: _rng.normal(s) * 0.05)(Dm, Df) * (Dm ** -0.5)),
            "w_down": _w((lambda *s: _rng.normal(s) * 0.05)(Df, Dm) * (Df ** -0.5)),
        }
    _B_in = _B_setup()

    return {
        "A_x": _A_in["x"],
        "A_wqkv": _A_in["wqkv"],
        "A_w_phi": _A_in["w_phi"],
        "A_wo": _A_in["wo"],
        "B_x": _B_in["x"],
        "B_w_gate": _B_in["w_gate"],
        "B_w_up": _B_in["w_up"],
        "B_w_down": _B_in["w_down"],
    }

def _fwd_reference(A_x, A_wqkv, A_w_phi, A_wo, B_x, B_w_gate, B_w_up, B_w_down):
    def _A_ref(x, wqkv, w_phi, wo):
        B, S, D = x.shape
        H = 16; Dh = D // H
        qkv = (lambda x, *d: x.transpose(*d))((x @ wqkv).reshape(B, S, 3, H, Dh), 2, 0, 3, 1, 4)
        q, k, v = qkv[0], qkv[1], qkv[2]
        pq = jnp.einsum("bhsd,hdf->bhsf", q, w_phi)
        pk = jnp.einsum("bhsd,hdf->bhsf", k, w_phi)
        phi_q = jnp.concatenate([_softmax(pq, axis=-1), _softmax(-pq, axis=-1)], axis=-1)
        phi_k = jnp.concatenate([_softmax(pk, axis=-1), _softmax(-pk, axis=-1)], axis=-1)
        kv = jnp.einsum("bhsf,bhsd->bhfd", phi_k, v)
        z  = jnp.einsum("bhsf->bhf", phi_k)
        num = jnp.einsum("bhqf,bhfd->bhqd", phi_q, kv)
        den = jnp.einsum("bhqf,bhf->bhq", phi_q, z)[..., None] + 1e-6
        o = num / den
        return (lambda x, *d: x.transpose(*d))(o, 0, 2, 1, 3).reshape(B, S, D) @ wo

    def _B_ref(x, w_gate, w_up, w_down):
        g = jnp.einsum("bsd,df->bsf", x, w_gate)
        u = jnp.einsum("bsd,df->bsf", x, w_up)
        h = _gelu(g) * u
        return jnp.einsum("bsf,fd->bsd", h, w_down)

    x = A_x
    xn = _layernorm(x, axis=-1)
    return x + _A_ref(xn, A_wqkv, A_w_phi, A_wo) + _B_ref(xn, B_w_gate, B_w_up, B_w_down)


def setup_inputs():
    _inp = _fwd_setup_inputs()
    _gk = jax.random.fold_in(jax.random.key(int.from_bytes(__import__("os").urandom(4), "little")), 2**31 - 1)
    _shapes = [[1, 2048, 448]]
    _dtypes = ['bfloat16']
    _gks = jax.random.split(_gk, len(_shapes))
    _gs = [jax.random.normal(k, s, dtype=jnp.dtype(d)) * 0.05 for k, s, d in zip(_gks, _shapes, _dtypes)]
    _inp["grad_out"] = _gs[0]
    return _inp

def reference(A_x, A_wqkv, A_w_phi, A_wo, B_w_gate, B_w_up, B_w_down, B_x, grad_out):
    _const = dict(B_x=B_x)
    def _f(*_d):
        return _fwd_reference(**{'A_x': _d[0], 'A_wqkv': _d[1], 'A_w_phi': _d[2], 'A_wo': _d[3], 'B_w_gate': _d[4], 'B_w_up': _d[5], 'B_w_down': _d[6], **_const})
    _out, _vjp = jax.vjp(_f, A_x, A_wqkv, A_w_phi, A_wo, B_w_gate, B_w_up, B_w_down)
    _grads = _vjp(grad_out)
    _out0 = jnp.asarray(_out)
    return (_out0, *[jnp.asarray(_g) for _g in _grads])
```

```python
import functools

import jax
import jax.numpy as jnp
import jax.experimental.pallas as pl
import jax.experimental.pallas.tpu as pltpu

F32 = jnp.float32
BF16 = jnp.bfloat16

S, D, H, DH, DF = 2048, 448, 16, 28, 1792
NG = H // 2
GR = 2 * DH
GE = 64
GF = 2 * GR
T = 512
NT_ = S // T
FC = 256
NF = DF // FC
LN_EPS = 1e-5
DEN_EPS = 1e-6
GELU_C1 = 0.7978845608028654
GELU_C2 = GELU_C1 * 0.044715


def _nn(a, b):
    return jnp.dot(a, b, preferred_element_type=F32)


def _nt(a, b):
    return jax.lax.dot_general(a, b, (((1,), (1,)), ((), ())),
                               preferred_element_type=F32)


def _iota(shape, dim):
    return jax.lax.broadcasted_iota(jnp.int32, shape, dim)


def _seg_reduce(p, op, red, fill):
    t = p.shape[-1]
    low = _iota((NG, 8, t), 1) < 4
    v = [p[:, 8 * i:8 * i + 8, :] for i in range(7)]
    a = op(op(v[0], v[1]), op(v[2], jnp.where(low, v[3], fill)))
    b = op(op(v[4], v[5]), op(v[6], jnp.where(low, fill, v[3])))
    return red(a, axis=1, keepdims=True), red(b, axis=1, keepdims=True)


def _seg_mix(ra, rb):
    t = ra.shape[-1]
    low = _iota((NG, 8, t), 1) < 4
    return jnp.where(low, ra, rb)


def _seg_expand(ra, rb):
    t = ra.shape[-1]
    a = jnp.broadcast_to(ra, (NG, 8, t))
    b = jnp.broadcast_to(rb, (NG, 8, t))
    return jnp.concatenate([a, a, a, _seg_mix(ra, rb), b, b, b], axis=1)


def _seg_sum(p):
    return _seg_reduce(p, jnp.add, jnp.sum, 0.0)


def _softmax_pair(p):
    mx = _seg_expand(*_seg_reduce(p, jnp.maximum, jnp.max, -jnp.inf))
    mn = _seg_expand(*_seg_reduce(p, jnp.minimum, jnp.min, jnp.inf))
    ep = jnp.exp(p - mx)
    en = jnp.exp(mn - p)
    pa, pb = _seg_sum(ep)
    na, nb = _seg_sum(en)
    return ep * _seg_expand(1.0 / pa, 1.0 / pb), en * _seg_expand(1.0 / na, 1.0 / nb)


def _softmax_pair_bwd(sp, sn, dsp, dsn):
    tp = sp * dsp
    tn = sn * dsn
    return (tp - sp * _seg_expand(*_seg_sum(tp))) - (tn - sn * _seg_expand(*_seg_sum(tn)))


def _head_blocks(acc):
    r = _iota((NG, GE, GF), 1)
    c = _iota((NG, GE, GF), 2)
    row_b = ((r >= DH) & (r < GR)) | (r >= GR + 4)
    col_b = ((c >= DH) & (c < GR)) | (c >= GR + DH)
    m = jnp.where(row_b == col_b, acc, 0.0)
    padded = jnp.concatenate([m, jnp.zeros((NG, GE, 128 - GF), F32)], axis=2)
    z = padded.reshape(NG * GE, 128).T
    lane_lo = _iota((GF, 128), 1) < GE
    pairs = []
    for p in range(NG // 2):
        zp = z[:GF, 128 * p:128 * p + 128]
        pairs.append(jnp.concatenate(
            [jnp.where(lane_lo, zp, 0.0), jnp.where(lane_lo, 0.0, zp)], axis=0))
    return m.astype(BF16), jnp.stack(pairs).astype(BF16)


def _ffn_elem(g, u, dh):
    g2 = g * g
    t = jnp.tanh(g * (GELU_C1 + GELU_C2 * g2))
    a = 0.5 + 0.5 * t
    ge = g * a
    h = ge * u
    gp = a + ge * (1.0 - a) * (2.0 * GELU_C1 + (6.0 * GELU_C2) * g2)
    dg = dh * u * gp
    du = dh * ge
    return h.astype(BF16), dg.astype(BF16), du.astype(BF16)


def _kernel(xT_h, dyT_h, wqkv_h, wphi_h, wo_h, wg_h, wu_h, wdT_h,
            outT_h, dxT_h, dwqkv_h, dwphi_h, dwo_h, dwg_h, dwu_h, dwdT_h,
            xT, dyT, wqkv, wphi, wo, wg, wu, wdT,
            xnT, xn, dy, rstd_s, doT, phik_s, vext_s, dp_s,
            wqkvT, WT, Wp, woT, accT, dxnT,
            outT, dxT, dwqkv, dwphi, dwo, dwg, dwu, dwdT,
            sem_in, sem_out):
    in_pairs = [(wphi_h, wphi), (wo_h, wo), (dyT_h, dyT), (wqkv_h, wqkv),
                (xT_h, xT), (wg_h, wg), (wu_h, wu), (wdT_h, wdT)]
    in_cp = [pltpu.make_async_copy(h, v, sem_in.at[n])
             for n, (h, v) in enumerate(in_pairs)]
    for cp in in_cp:
        cp.start()
    out_cp = []

    def send(src, dst):
        cp = pltpu.make_async_copy(src, dst, sem_out.at[len(out_cp)])
        cp.start()
        out_cp.append(cp)

    cols = lambda i: slice(i * T, (i + 1) * T)

    in_cp[0].wait()
    r = _iota((D, D), 0)
    c = _iota((D, D), 1)
    perm = jnp.where(r == (c & 15) * DH + (c >> 4), 1.0, 0.0).astype(BF16)
    perm_t = jnp.where(c == (r & 15) * DH + (r >> 4), 1.0, 0.0).astype(BF16)
    wphi_hd = _nn(perm, wphi[...]).astype(BF16)
    rr = _iota((GF, DH), 0)
    rc = _iota((GF, DH), 1)
    rep = jnp.where((rr == rc) | (rr == rc + DH) | (rr == rc + 2 * DH) | (rr == rc + 3 * DH),
                    1.0, 0.0).astype(BF16)
    br = _iota((GF, GF), 0)
    bc = _iota((GF, GF), 1)
    blk = lambda t: ((t >= DH).astype(jnp.int32) + (t >= 2 * DH).astype(jnp.int32)
                     + (t >= 3 * DH).astype(jnp.int32))
    diag = blk(br) == blk(bc)
    phi_t = [jnp.where(diag, _nt(rep, wphi_hd[GF * g:GF * g + GF]), 0.0).astype(BF16)
             for g in range(4)]
    phi_n = [jnp.where(diag, _nt(wphi_hd[GF * g:GF * g + GF], rep), 0.0).astype(BF16)
             for g in range(4)]

    in_cp[1].wait()
    in_cp[2].wait()
    woT[...] = wo[...].T
    for i in range(NT_):
        dyt = dyT[:, cols(i)]
        doT[:, cols(i)] = _nn(wo[...], dyt)
        dy[cols(i), :] = dyt.T

    in_cp[3].wait()
    wqkvT[...] = wqkv[...].T
    for g in range(8):
        WT[GF * g:GF * g + GF, :] = _nn(phi_t[g % 4], wqkvT[GF * g:GF * g + GF, :]).astype(BF16)
    WT[2 * D:, :] = wqkvT[2 * D:, :]
    Wp[:, :2 * D] = WT[:2 * D, :].T
    Wp[:, 2 * D:] = wqkv[:, 2 * D:]

    in_cp[4].wait()
    kv_acc = [None] * NG
    for i in range(NT_):
        x = xT[:, cols(i)].astype(F32)
        xc = x - jnp.mean(x, axis=0, keepdims=True)
        rstd = jax.lax.rsqrt(jnp.mean(xc * xc, axis=0, keepdims=True) + LN_EPS)
        xb = (xc * rstd).astype(BF16)
        rstd_s[:, cols(i)] = rstd
        xnT[:, cols(i)] = xb
        xn[cols(i), :] = xb.T
        pkv = _nn(WT[D:, :], xb)
        sp, sn = _softmax_pair(pkv[:D].reshape(NG, GR, T))
        phik = jnp.concatenate([sp, sn], axis=1).astype(BF16)
        vext = jnp.concatenate([pkv[D:].reshape(NG, GR, T), jnp.ones((NG, 8, T), F32)],
                               axis=1).astype(BF16)
        phik_s[:, :, cols(i)] = phik
        vext_s[:, :, cols(i)] = vext
        for j in range(NG):
            part = _nt(vext[j], phik[j])
            kv_acc[j] = part if i == 0 else kv_acc[j] + part
    kvT, kvP = _head_blocks(jnp.stack(kv_acc))

    in_cp[5].wait()
    in_cp[6].wait()
    in_cp[7].wait()
    for j in range(NF):
        fc = slice(j * FC, (j + 1) * FC)
        wgc, wuc, wdc = wg[:, fc], wu[:, fc], wdT[:, fc]
        g = _nn(xn[...], wgc)
        u = _nn(xn[...], wuc)
        dh = _nn(dy[...], wdc)
        h, dg, du = _ffn_elem(g, u, dh)
        po = _nt(wdc, h)
        px = _nt(wgc, dg) + _nt(wuc, du)
        if j == 0:
            accT[...] = po
            dxnT[...] = px
        else:
            accT[...] += po
            dxnT[...] += px
        dwg[:, fc] = _nn(xnT[...], dg).astype(BF16)
        dwu[:, fc] = _nn(xnT[...], du).astype(BF16)
        dwdT[:, fc] = _nn(dyT[...], h).astype(BF16)
    send(dwg, dwg_h)
    send(dwu, dwu_h)
    send(dwdT, dwdT_h)

    dkv_acc = [None] * NG
    dwo_acc = None
    low = _iota((NG, 8, T), 1) < 4
    for i in range(NT_):
        pq = _nn(WT[:D, :], xnT[:, cols(i)])
        sp, sn = _softmax_pair(pq.reshape(NG, GR, T))
        phiq = jnp.concatenate([sp, sn], axis=1).astype(BF16)
        ne = jnp.stack([_nn(kvT[j], phiq[j]) for j in range(NG)])
        rmix = 1.0 / (ne[:, GR:, :] + DEN_EPS)
        rrot = pltpu.roll(rmix, 4, 1)
        ra = jnp.where(low, rmix, rrot)
        rb = jnp.where(low, rrot, rmix)
        rden = jnp.concatenate([ra, ra, ra, rmix, rb, rb, rb], axis=1)
        o = ne[:, :GR, :] * rden
        dnum = doT[:, cols(i)].reshape(NG, GR, T) * rden
        dden = _seg_mix(*_seg_sum(dnum * o)) * (-0.25)
        dne = jnp.concatenate([dnum, dden], axis=1).astype(BF16)
        ob = o.reshape(D, T).astype(BF16)
        outT[:, cols(i)] = (xT[:, cols(i)].astype(F32) + accT[:, cols(i)]
                            + _nn(woT[...], ob)).astype(BF16)
        part = _nt(ob, dyT[:, cols(i)])
        dwo_acc = part if i == 0 else dwo_acc + part
        dphi = jnp.stack([_nn(kvP[p], dne[2 * p:2 * p + 2].reshape(2 * GE, T))
                          for p in range(NG // 2)]).reshape(NG, GF, T)
        for j in range(NG):
            part = _nt(dne[j], phiq[j])
            dkv_acc[j] = part if i == 0 else dkv_acc[j] + part
        dpq = _softmax_pair_bwd(sp, sn, dphi[:, :GR, :], dphi[:, GR:, :])
        dp_s[:D, cols(i)] = dpq.reshape(D, T).astype(BF16)
    dwo[...] = dwo_acc.astype(BF16)
    send(outT, outT_h)
    send(dwo, dwo_h)
    dkvT, dkvP = _head_blocks(jnp.stack(dkv_acc))

    g_acc = None
    for i in range(NT_):
        phik = phik_s[:, :, cols(i)]
        vext = vext_s[:, :, cols(i)]
        dphi = jnp.stack([_nn(dkvP[p], vext[2 * p:2 * p + 2].reshape(2 * GE, T))
                          for p in range(NG // 2)]).reshape(NG, GF, T)
        dv = jnp.stack([_nn(dkvT[j], phik[j])[:GR] for j in range(NG)])
        pf = phik.astype(F32)
        dpk = _softmax_pair_bwd(pf[:, :GR, :], pf[:, GR:, :], dphi[:, :GR, :], dphi[:, GR:, :])
        dp_s[D:2 * D, cols(i)] = dpk.reshape(D, T).astype(BF16)
        dp_s[2 * D:, cols(i)] = dv.reshape(D, T).astype(BF16)
        dp = dp_s[:, cols(i)]
        xb = xnT[:, cols(i)]
        part = _nt(xb, dp)
        g_acc = part if i == 0 else g_acc + part
        dxn = dxnT[:, cols(i)] + _nn(Wp[...], dp)
        xf = xb.astype(F32)
        m1 = jnp.mean(dxn, axis=0, keepdims=True)
        m2 = jnp.mean(dxn * xf, axis=0, keepdims=True)
        dxT[:, cols(i)] = (dyT[:, cols(i)].astype(F32)
                           + (dxn - m1 - xf * m2) * rstd_s[:, cols(i)]).astype(BF16)
    send(dxT, dxT_h)

    gb = g_acc.astype(BF16)
    gT = gb[:, :2 * D].T
    dwT = jnp.concatenate([_nn(phi_n[g % 4], gT[GF * g:GF * g + GF]).astype(BF16)
                           for g in range(8)], axis=0)
    dwqkv[:, :2 * D] = dwT.T
    dwqkv[:, 2 * D:] = gb[:, 2 * D:]
    send(dwqkv, dwqkv_h)
    ys = []
    for g in range(4):
        xq = _nt(wqkvT[GF * g:GF * g + GF, :], gT[GF * g:GF * g + GF])
        xk = _nt(wqkvT[D + GF * g:D + GF * g + GF, :], gT[D + GF * g:D + GF * g + GF])
        ys.append(_nn(jnp.where(diag, xq + xk, 0.0).astype(BF16), rep).astype(BF16))
    dwphi[...] = _nn(perm_t, jnp.concatenate(ys, axis=0)).astype(BF16)
    send(dwphi, dwphi_h)

    for cp in out_cp:
        cp.wait()


@jax.jit
def pallas_parallel_sum__linear_kernel_hedgehog__glu_gated_geglu__prompt_kernel(
    A_x: jax.Array,
    A_wqkv: jax.Array,
    A_w_phi: jax.Array,
    A_wo: jax.Array,
    B_x: jax.Array,
    B_w_gate: jax.Array,
    B_w_up: jax.Array,
    B_w_down: jax.Array,
    grad_out: jax.Array,
):
    del B_x
    xT = A_x.reshape(S, D).T
    dyT = grad_out.reshape(S, D).T
    wphi = A_w_phi.transpose(1, 0, 2).reshape(DH * H, DH)
    wdT = B_w_down.T

    vm = pltpu.VMEM
    sds = lambda *s: jax.ShapeDtypeStruct(s, BF16)
    out_shape = (sds(D, S), sds(D, S), sds(D, 3 * D), sds(D, DH), sds(D, D),
                 sds(D, DF), sds(D, DF), sds(D, DF))
    scratch = [
        vm((D, S), BF16), vm((D, S), BF16), vm((D, 3 * D), BF16), vm((D, DH), BF16),
        vm((D, D), BF16), vm((D, DF), BF16), vm((D, DF), BF16), vm((D, DF), BF16),
        vm((D, S), BF16), vm((S, D), BF16), vm((S, D), BF16), vm((1, S), F32),
        vm((D, S), F32), vm((NG, GF, S), BF16), vm((NG, GE, S), BF16), vm((3 * D, S), BF16),
        vm((3 * D, D), BF16), vm((3 * D, D), BF16), vm((D, 3 * D), BF16), vm((D, D), BF16),
        vm((D, S), F32), vm((D, S), F32),
        vm((D, S), BF16), vm((D, S), BF16), vm((D, 3 * D), BF16), vm((D, DH), BF16),
        vm((D, D), BF16), vm((D, DF), BF16), vm((D, DF), BF16), vm((D, DF), BF16),
        pltpu.SemaphoreType.DMA((8,)), pltpu.SemaphoreType.DMA((8,)),
    ]
    any_spec = pl.BlockSpec(memory_space=pl.ANY)
    outT, dxT, dwqkv, dwphi, dwo, dwg, dwu, dwdT = pl.pallas_call(
        _kernel,
        out_shape=out_shape,
        in_specs=[any_spec] * 8,
        out_specs=[any_spec] * 8,
        scratch_shapes=scratch,
        compiler_params=pltpu.CompilerParams(vmem_limit_bytes=120 * 1024 * 1024),
    )(xT, dyT, A_wqkv, wphi, A_wo, B_w_gate, B_w_up, wdT)

    return (outT.T.reshape(1, S, D), dxT.T.reshape(1, S, D), dwqkv,
            dwphi.reshape(DH, H, DH).transpose(1, 0, 2), dwo, dwg, dwu, dwdT.T)
```

```python
import jax
import jax.numpy as jnp
import jax.experimental.pallas as pl
import jax.experimental.pallas.tpu as pltpu

F32 = jnp.float32
BF16 = jnp.bfloat16

S, D, H, DH, DF = 2048, 448, 16, 28, 1792
NG = H // 2
GR = 2 * DH
GE = 64
GF = 2 * GR
T = 512
TH = T // 2
NT_ = S // T
NP = S // 2
DA, DB = 256, 192
DM = D // 2
MB = 512
NM = NP // MB
CH = ((0, 256), (512, 256), (1024, 256), (1536, 128))
XF_W = 4 * DA + 9 * 128
LN_EPS = 1e-5
DEN_EPS = 1e-6
GELU_C1 = 0.7978845608028654
GELU_C2 = GELU_C1 * 0.044715


def _nn(a, b):
    return jnp.dot(a, b, preferred_element_type=F32)


def _nt(a, b):
    return jax.lax.dot_general(a, b, (((1,), (1,)), ((), ())),
                               preferred_element_type=F32)


def _iota(shape, dim):
    return jax.lax.broadcasted_iota(jnp.int32, shape, dim)


def _rows(*parts):
    return jnp.concatenate(parts, axis=0)


def _lanes(*parts):
    return jnp.concatenate(parts, axis=1)


def _seg_reduce(p, op, red, fill):
    t = p.shape[-1]
    low = _iota((NG, 8, t), 1) < 4
    v = [p[:, 8 * i:8 * i + 8, :] for i in range(7)]
    a = op(op(v[0], v[1]), op(v[2], jnp.where(low, v[3], fill)))
    b = op(op(v[4], v[5]), op(v[6], jnp.where(low, fill, v[3])))
    return red(a, axis=1, keepdims=True), red(b, axis=1, keepdims=True)


def _seg_mix(ra, rb):
    t = ra.shape[-1]
    low = _iota((NG, 8, t), 1) < 4
    return jnp.where(low, ra, rb)


def _seg_expand(ra, rb):
    t = ra.shape[-1]
    a = jnp.broadcast_to(ra, (NG, 8, t))
    b = jnp.broadcast_to(rb, (NG, 8, t))
    return jnp.concatenate([a, a, a, _seg_mix(ra, rb), b, b, b], axis=1)


def _seg_sum(p):
    return _seg_reduce(p, jnp.add, jnp.sum, 0.0)


def _softmax_pair(p):
    mx = _seg_expand(*_seg_reduce(p, jnp.maximum, jnp.max, -jnp.inf))
    mn = _seg_expand(*_seg_reduce(p, jnp.minimum, jnp.min, jnp.inf))
    ep = jnp.exp(p - mx)
    en = jnp.exp(mn - p)
    pa, pb = _seg_sum(ep)
    na, nb = _seg_sum(en)
    return ep * _seg_expand(1.0 / pa, 1.0 / pb), en * _seg_expand(1.0 / na, 1.0 / nb)


def _softmax_pair_bwd(sp, sn, dsp, dsn):
    tp = sp * dsp
    tn = sn * dsn
    return (tp - sp * _seg_expand(*_seg_sum(tp))) - (tn - sn * _seg_expand(*_seg_sum(tn)))


def _head_blocks(acc):
    r = _iota((NG, GE, GF), 1)
    c = _iota((NG, GE, GF), 2)
    row_b = ((r >= DH) & (r < GR)) | (r >= GR + 4)
    col_b = ((c >= DH) & (c < GR)) | (c >= GR + DH)
    m = jnp.where(row_b == col_b, acc, 0.0)
    padded = jnp.concatenate([m, jnp.zeros((NG, GE, 128 - GF), F32)], axis=2)
    z = padded.reshape(NG * GE, 128).T
    lane_lo = _iota((GF, 128), 1) < GE
    pairs = []
    for p in range(NG // 2):
        zp = z[:GF, 128 * p:128 * p + 128]
        pairs.append(jnp.concatenate(
            [jnp.where(lane_lo, zp, 0.0), jnp.where(lane_lo, 0.0, zp)], axis=0))
    return m.astype(BF16), jnp.stack(pairs).astype(BF16)


def _ffn_elem(g, u, dh):
    g2 = g * g
    t = jnp.tanh(g * (GELU_C1 + GELU_C2 * g2))
    a = 0.5 + 0.5 * t
    ge = g * a
    h = ge * u
    gp = a + ge * (1.0 - a) * (2.0 * GELU_C1 + (6.0 * GELU_C2) * g2)
    dg = dh * u * gp
    du = dh * ge
    return h, dg, du


def _head_add(a, b):
    n = b.shape[0]
    return _rows(a[:n] + b, a[n:])


def _head_sub(a, b):
    n = b.shape[0]
    return _rows(a[:n] - b, a[n:])


def _x_fwd_ops(x):
    lo, hi = x[:, :TH], x[:, TH:]
    x11, x12, x21, x22 = lo[:DA], lo[DA:], hi[:DA], hi[DA:]
    ops = [_head_add(x11, x22), _head_add(x21, x22), x11, x22,
           x11[:DB] + x12, x21 - x11, x12 - x22]
    return [o.astype(BF16) for o in ops]


def _x_row_ops(x):
    lo, hi = x[:, :TH], x[:, TH:]
    x11, x12, x21, x22 = lo[:DM], lo[DM:], hi[:DM], hi[DM:]
    ops = [x11 + x22, x21 + x22, x11, x22, x11 + x12, x21 - x11, x12 - x22]
    return [o.astype(BF16) for o in ops]


def _w_fwd_ops(lo, hi):
    w11, w12, w21, w22 = lo[:DA], hi[:DA], lo[DA:], hi[DA:]
    return [_head_add(w11, w22), w11, _head_sub(w12, w22), w21 - w11[:DB],
            w22, w11 + w12, w21 + w22]


def _w_row_ops(lo, hi):
    w11, w12, w21, w22 = lo[:DM], hi[:DM], lo[DM:], hi[DM:]
    ops = [w11 + w22, w11, w12 - w22, w21 - w11, w22, w11 + w12, w21 + w22]
    return [o.astype(BF16) for o in ops]


def _y_ops(y11, y12, y21, y22):
    ops = [y11 + y22, y21 - y22, y12 + y22, y11 + y21, y12 - y11, y22, y11]
    return [o.astype(BF16) for o in ops]


def _y_from(p):
    return (p[0] + p[3] - p[4] + p[6], p[2] + p[4], p[1] + p[3],
            p[0] - p[1] + p[2] + p[5])


def _x_from(p):
    return (p[0] + p[2] + p[4] - p[5], p[4] + p[6], p[1] + p[5],
            p[0] + p[1] + p[3] - p[6])


def _w_from(p):
    return (p[0] + p[1] - p[3] + p[5], p[2] + p[5], p[3] + p[6],
            p[0] - p[2] + p[4] + p[6])


def _tri_left(a):
    return [a[0:128], a[64:192], _rows(a[0:64], a[128:192])]


def _tri_right(b):
    b1, b2 = b[:, :128], b[:, 128:]
    return [_rows(b1[0:64], b2[64:128]),
            _rows(b1[64:128] - b2[64:128], b1[128:192]),
            _rows(b2[0:64] - b1[0:64], b2[128:192])]


_SHORT = (3, 4, 6)
_XF_OFF = {0: 0, 1: DA, 2: 2 * DA, 5: 3 * DA,
           3: 4 * DA, 4: 4 * DA + 384, 6: 4 * DA + 768}


def _kernel(xT_h, dyT_h, wqkv_h, wphi_h, wo_h, wg_h, wu_h, wdT_h,
            outT_h, dxT_h, dwqkv_h, dwphi_h, dwo_h, dwg_h, dwu_h, dwdT_h,
            xT, dyT, wqkv, wphi, wo, wg, wu, wdT,
            xnT, xf_s, xw_s, phik_s, vext_s, dp_s,
            wqkvT, WT, Wp, woT,
            outT, dxT, dwqkv, dwphi, dwo, dwg, dwu, dwdT,
            sem_in, sem_out):
    cols = lambda i: slice(i * T, (i + 1) * T)
    prs = lambda i: slice(i * TH, (i + 1) * TH)
    blk = lambda m: slice(m * MB, (m + 1) * MB)

    in_list = [
        ("wo", wo_h, wo),
        ("dy0", dyT_h.at[:, cols(0)], dyT.at[:, cols(0)]),
        ("dy1", dyT_h.at[:, T:], dyT.at[:, T:]),
        ("wd", wdT_h, wdT),
        ("x", xT_h, xT),
        ("wphi", wphi_h, wphi),
        ("wqkv", wqkv_h, wqkv),
        ("wg", wg_h, wg),
        ("wu", wu_h, wu),
    ]
    in_cp = {}
    for n, (name, h, v) in enumerate(in_list):
        in_cp[name] = pltpu.make_async_copy(h, v, sem_in.at[n])
        in_cp[name].start()
    out_cp = []

    def send(src, dst):
        cp = pltpu.make_async_copy(src, dst, sem_out.at[len(out_cp)])
        cp.start()
        out_cp.append(cp)

    V = {}

    def acc(key, val):
        V[key] = V[key] + val if key in V else val

    def wait(*names):
        for n in names:
            in_cp[n].wait()

    def prep_x(which, i, x):
        for n, op in enumerate(_x_fwd_ops(x)):
            pieces = _tri_left(op) if n in _SHORT else [op]
            off = _XF_OFF[n]
            for pc in pieces:
                xf_s[which, prs(i), off:off + pc.shape[0]] = pc.T
                off += pc.shape[0]
        for n, op in enumerate(_x_row_ops(x)):
            xw_s[which, n, :, prs(i)] = op

    def prep_w(name, ref, c):
        c0, w = CH[c]
        lo = ref[:, c0:c0 + w].astype(F32)
        hi = ref[:, c0 + w:c0 + 2 * w].astype(F32)
        fw = []
        for n, op in enumerate(_w_fwd_ops(lo, hi)):
            if n not in _SHORT:
                fw.append([op.astype(BF16)])
            elif w == 256:
                fw.append([o.astype(BF16) for o in _tri_right(op)])
            else:
                fw.append([_rows(op[:128], jnp.zeros((64, w), F32), op[128:]).astype(BF16)])
        V["wf", name, c] = fw
        V["wr", name, c] = _w_row_ops(lo, hi)

    def fwd(which, names, c, m, n):
        w = CH[c][1]
        off = _XF_OFF[n]
        rhs = [_lanes(*parts) for parts in zip(*[V["wf", nm, c][n] for nm in names])]
        if len(rhs) == 1:
            p = _nn(xf_s[which, blk(m), off:off + DA], rhs[0])
            for k, nm in enumerate(names):
                V["p", nm, c, m, n] = p[:, k * w:(k + 1) * w]
        else:
            e, n1, n2 = [_nn(xf_s[which, blk(m), off + 128 * k:off + 128 * k + 128], rhs[k])
                         for k in range(3)]
            for k, nm in enumerate(names):
                sl = slice(128 * k, 128 * k + 128)
                V["p", nm, c, m, n] = _lanes(e[:, sl] + n1[:, sl], e[:, sl] + n2[:, sl])

    def elem(c, m):
        g, u, dh = [_y_from([V.pop(("p", nm, c, m, n)) for n in range(7)])
                    for nm in ("g", "u", "d")]
        h, dg, du = zip(*[_ffn_elem(*t) for t in zip(g, u, dh)])
        V["y", 1, c, m] = _y_ops(*h)
        V["y", 0, c, m] = [_lanes(a, b) for a, b in zip(_y_ops(*dg), _y_ops(*du))]

    def bwd_x(which, names, c, m, n):
        lhs = _lanes(*[V["wr", nm, c][n] for nm in names])
        acc(("ax", which, m, n), _nt(lhs, V["y", which, c, m][n]))

    def bwd_w(which, c, m, n):
        acc(("aw", which, c, n), _nn(xw_s[which, n, :, blk(m)], V["y", which, c, m][n]))

    def fin_w(which, c):
        c0, w = CH[c]
        q = _w_from([V.pop(("aw", which, c, n)) for n in range(7)])
        refs = ((dwg, dwg_h), (dwu, dwu_h)) if which == 0 else ((dwdT, dwdT_h),)
        for k, (ref, hbm) in enumerate(refs):
            sl = slice(k * w, (k + 1) * w)
            ref[:DM, c0:c0 + w] = q[0][:, sl].astype(BF16)
            ref[:DM, c0 + w:c0 + 2 * w] = q[1][:, sl].astype(BF16)
            ref[DM:, c0:c0 + w] = q[2][:, sl].astype(BF16)
            ref[DM:, c0 + w:c0 + 2 * w] = q[3][:, sl].astype(BF16)
            send(ref.at[:, c0:c0 + 2 * w], hbm.at[:, c0:c0 + 2 * w])

    def ffn_x(which, i):
        m, j = divmod(i * TH, MB)
        q = _x_from([V["ax", which, m, n][:, j:j + TH] for n in range(7)])
        return _lanes(_rows(q[0], q[1]), _rows(q[2], q[3]))

    def consts():
        r = _iota((D, D), 0)
        c = _iota((D, D), 1)
        V["perm"] = jnp.where(r == (c & 15) * DH + (c >> 4), 1.0, 0.0).astype(BF16)
        V["perm_t"] = jnp.where(c == (r & 15) * DH + (r >> 4), 1.0, 0.0).astype(BF16)
        rr = _iota((GF, DH), 0)
        rc = _iota((GF, DH), 1)
        V["rep"] = jnp.where((rr == rc) | (rr == rc + DH) | (rr == rc + 2 * DH) | (rr == rc + 3 * DH),
                             1.0, 0.0).astype(BF16)
        br = _iota((GF, GF), 0)
        bc = _iota((GF, GF), 1)
        bi = lambda t: ((t >= DH).astype(jnp.int32) + (t >= 2 * DH).astype(jnp.int32)
                        + (t >= 3 * DH).astype(jnp.int32))
        V["diag"] = jnp.where(bi(br) == bi(bc), 1.0, 0.0)

    def do_mm(i):
        dyt = dyT[:, cols(i)]
        V["do", i] = _nn(wo[...], dyt)
        prep_x(1, i, dyt.astype(F32))

    def phi_a():
        V["wphi_hd"] = _nn(V["perm"], wphi[...]).astype(BF16)
        wqkvT[...] = wqkv[...].T
        woT[...] = wo[...].T

    def phi_b():
        whd, rep, diag = V["wphi_hd"], V["rep"], V["diag"] > 0.5
        V["phi_t"] = [jnp.where(diag, _nt(rep, whd[GF * g:GF * g + GF]), 0.0).astype(BF16)
                      for g in range(4)]
        V["phi_n"] = [jnp.where(diag, _nt(whd[GF * g:GF * g + GF], rep), 0.0).astype(BF16)
                      for g in range(4)]

    def fold():
        for g in range(8):
            WT[GF * g:GF * g + GF, :] = _nn(V["phi_t"][g % 4],
                                            wqkvT[GF * g:GF * g + GF, :]).astype(BF16)
        WT[2 * D:, :] = wqkvT[2 * D:, :]
        Wp[:, :2 * D] = WT[:2 * D, :].T
        Wp[:, 2 * D:] = wqkv[:, 2 * D:]

    def ln(i):
        x = xT[:, cols(i)].astype(F32)
        xc = x - jnp.mean(x, axis=0, keepdims=True)
        rstd = jax.lax.rsqrt(jnp.mean(xc * xc, axis=0, keepdims=True) + LN_EPS)
        xn = xc * rstd
        V["rstd", i] = rstd
        xnT[:, cols(i)] = xn.astype(BF16)
        prep_x(0, i, xn)

    def k_fwd(i):
        pkv = _nn(WT[D:, :], xnT[:, cols(i)])
        sp, sn = _softmax_pair(pkv[:D].reshape(NG, GR, T))
        phik_s[:, :, cols(i)] = jnp.concatenate([sp, sn], axis=1).astype(BF16)
        vext_s[:, :, cols(i)] = jnp.concatenate(
            [pkv[D:].reshape(NG, GR, T), jnp.ones((NG, 8, T), F32)], axis=1).astype(BF16)

    def k_state(i):
        for j in range(NG):
            acc(("kv", j), _nt(vext_s[j, :, cols(i)], phik_s[j, :, cols(i)]))
        if i == NT_ - 1:
            V["kvT"], V["kvP"] = _head_blocks(jnp.stack([V.pop(("kv", j)) for j in range(NG)]))

    def q_fwd(i):
        pq = _nn(WT[:D, :], xnT[:, cols(i)])
        sp, sn = _softmax_pair(pq.reshape(NG, GR, T))
        V["sq", i] = (sp, sn)
        V["phiq", i] = jnp.concatenate([sp, sn], axis=1).astype(BF16)

    def q_mid(i):
        phiq = V["phiq", i]
        low = _iota((NG, 8, T), 1) < 4
        ne = jnp.stack([_nn(V["kvT"][j], phiq[j]) for j in range(NG)])
        rmix = 1.0 / (ne[:, GR:, :] + DEN_EPS)
        rrot = pltpu.roll(rmix, 4, 1)
        ra = jnp.where(low, rmix, rrot)
        rb = jnp.where(low, rrot, rmix)
        rden = jnp.concatenate([ra, ra, ra, rmix, rb, rb, rb], axis=1)
        o = ne[:, :GR, :] * rden
        dnum = V.pop(("do", i)).reshape(NG, GR, T) * rden
        dden = _seg_mix(*_seg_sum(dnum * o)) * (-0.25)
        V["dne", i] = jnp.concatenate([dnum, dden], axis=1).astype(BF16)
        V["ob", i] = o.reshape(D, T).astype(BF16)

    def q_bwd(i):
        dne, phiq = V.pop(("dne", i)), V.pop(("phiq", i))
        dphi = jnp.stack([_nn(V["kvP"][p], dne[2 * p:2 * p + 2].reshape(2 * GE, T))
                          for p in range(NG // 2)]).reshape(NG, GF, T)
        for j in range(NG):
            acc(("dkv", j), _nt(dne[j], phiq[j]))
        sp, sn = V.pop(("sq", i))
        dpq = _softmax_pair_bwd(sp, sn, dphi[:, :GR, :], dphi[:, GR:, :])
        dp_s[:D, cols(i)] = dpq.reshape(D, T).astype(BF16)
        if i == NT_ - 1:
            V["dkvT"], V["dkvP"] = _head_blocks(jnp.stack([V.pop(("dkv", j)) for j in range(NG)]))

    def dwo_mm(i):
        acc("dwo", _nt(V["ob", i], dyT[:, cols(i)]))
        if i == NT_ - 1:
            dwo[...] = V.pop("dwo").astype(BF16)
            send(dwo, dwo_h)

    def k_bwd(i):
        phik = phik_s[:, :, cols(i)]
        vext = vext_s[:, :, cols(i)]
        dphi = jnp.stack([_nn(V["dkvP"][p], vext[2 * p:2 * p + 2].reshape(2 * GE, T))
                          for p in range(NG // 2)]).reshape(NG, GF, T)
        dv = jnp.stack([_nn(V["dkvT"][j], phik[j])[:GR] for j in range(NG)])
        pf = phik.astype(F32)
        dpk = _softmax_pair_bwd(pf[:, :GR, :], pf[:, GR:, :], dphi[:, :GR, :], dphi[:, GR:, :])
        dp_s[D:2 * D, cols(i)] = dpk.reshape(D, T).astype(BF16)
        dp_s[2 * D:, cols(i)] = dv.reshape(D, T).astype(BF16)

    def g_mm(i):
        acc("G", _nt(xnT[:, cols(i)], dp_s[:, cols(i)]))

    def fin_out(i):
        outT[:, cols(i)] = (xT[:, cols(i)].astype(F32) + ffn_x(1, i)
                            + _nn(woT[...], V["ob", i])).astype(BF16)
        send(outT.at[:, cols(i)], outT_h.at[:, cols(i)])

    def fin_dx(i):
        dxn = ffn_x(0, i) + _nn(Wp[...], dp_s[:, cols(i)])
        xf = xnT[:, cols(i)].astype(F32)
        m1 = jnp.mean(dxn, axis=0, keepdims=True)
        m2 = jnp.mean(dxn * xf, axis=0, keepdims=True)
        dxT[:, cols(i)] = (dyT[:, cols(i)].astype(F32)
                           + (dxn - m1 - xf * m2) * V["rstd", i]).astype(BF16)
        send(dxT.at[:, cols(i)], dxT_h.at[:, cols(i)])

    def unfold_a():
        gb = V.pop("G").astype(BF16)
        V["gT"] = gb[:, :2 * D].T
        dwqkv[:, 2 * D:] = gb[:, 2 * D:]

    def unfold_b():
        gT = V["gT"]
        dwT = _rows(*[_nn(V["phi_n"][g % 4], gT[GF * g:GF * g + GF]).astype(BF16)
                      for g in range(8)])
        dwqkv[:, :2 * D] = dwT.T
        send(dwqkv, dwqkv_h)
        diag = V["diag"] > 0.5
        V["xqk"] = []
        for g in range(4):
            xq = _nt(wqkvT[GF * g:GF * g + GF, :], gT[GF * g:GF * g + GF])
            xk = _nt(wqkvT[D + GF * g:D + GF * g + GF, :], gT[D + GF * g:D + GF * g + GF])
            V["xqk"].append(jnp.where(diag, xq + xk, 0.0).astype(BF16))

    def unfold_c():
        V["ys"] = _rows(*[_nn(t, V["rep"]).astype(BF16) for t in V.pop("xqk")])

    def unfold_d():
        dwphi[...] = _nn(V["perm_t"], V.pop("ys")).astype(BF16)
        send(dwphi, dwphi_h)

    GU = ("g", "u")

    def t_fd(c, m):
        cost = MB * CH[c][1] // 256
        return [(cost * (0.75 if (n in _SHORT and CH[c][1] == 256) else 1.0),
                 lambda n=n: fwd(1, ("d",), c, m, n)) for n in range(7)]

    def t_fgu(c, m):
        cost = 2 * MB * CH[c][1] // 256
        return ([(cost * (0.75 if (n in _SHORT and CH[c][1] == 256) else 1.0),
                  lambda n=n: fwd(0, GU, c, m, n)) for n in range(7)]
                + [(0, lambda: elem(c, m))])

    def t_x(c, m):
        cost = 7 * MB * CH[c][1] // 2048
        return ([(cost, lambda n=n: bwd_x(1, ("d",), c, m, n)) for n in range(7)]
                + [(2 * cost, lambda n=n: bwd_x(0, GU, c, m, n)) for n in range(7)])

    def t_w(which, c, m):
        cost = 7 * MB * CH[c][1] // 2048 * (2 - which)
        t = [(cost, lambda n=n: bwd_w(which, c, m, n)) for n in range(7)]
        if m == NM - 1:
            t.append((0, lambda: fin_w(which, c)))
        return t

    def run(tasks):
        for _, fn in tasks:
            fn()

    def merge(back, extra):
        extra = sorted(extra, key=lambda e: e[0])
        pos = 0
        for cost, fn in back:
            while extra and extra[0][0] <= pos:
                extra.pop(0)[1]()
            fn()
            pos += cost
        for _, fn in extra:
            fn()

    consts()
    wait("wo", "dy0")
    do_mm(0)
    wait("dy1")
    for i in range(1, NT_):
        do_mm(i)
    wait("wd")
    for c in range(2):
        prep_w("d", wdT, c)
        run(t_fd(c, 0) + t_fd(c, 1))
    wait("x", "wphi", "wqkv", "wg", "wu")
    phi_a()
    prep_w("d", wdT, 2)
    prep_w("d", wdT, 3)
    for i in range(NT_):
        ln(i)
    prep_w("g", wg, 0)
    prep_w("u", wu, 0)
    steps = [(c, m) for c in range(len(CH)) for m in range(NM)]
    back = t_fd(2, 0) + t_fd(2, 1) + t_fd(3, 0) + t_fd(3, 1)
    back += t_fgu(*steps[0])
    late = []
    for k, (c, m) in enumerate(steps):
        if k + 1 < len(steps):
            cn, mn = steps[k + 1]
            if mn == 0:
                back.append((0, lambda cn=cn: (prep_w("g", wg, cn), prep_w("u", wu, cn))))
            back += t_fgu(cn, mn)
        else:
            back += late.pop(0)
        back += t_x(c, m)
        tw = t_w(0, c, m) + t_w(1, c, m)
        if c < 2 or (c == 2 and m == 0):
            back += tw
        else:
            late.append(tw)
    extra = [(1000, phi_b), (2500, fold)]
    p0, dp = 9000, 4000
    seq = ([(k_fwd, 0), (k_fwd, 1), (k_state, 0), (k_fwd, 2), (k_state, 1), (k_fwd, 3),
            (k_state, 2), (q_fwd, 0), (k_state, 3), (q_fwd, 1), (q_mid, 0), (q_fwd, 2)]
           + [(q_bwd, 0), (q_mid, 1), (dwo_mm, 0), (q_fwd, 3), (q_bwd, 1), (q_mid, 2), (dwo_mm, 1),
              (q_bwd, 2), (q_mid, 3), (dwo_mm, 2), (q_bwd, 3), (dwo_mm, 3)]
           + [(k_bwd, 0), (k_bwd, 1), (g_mm, 0), (k_bwd, 2), (g_mm, 1), (k_bwd, 3), (g_mm, 2),
              (g_mm, 3)])
    for k, (fn, i) in enumerate(seq):
        extra.append((p0 + dp * k, lambda fn=fn, i=i: fn(i)))
    k = len(seq)
    extra += [(p0 + dp * k, unfold_a), (p0 + dp * k + 2000, unfold_b),
              (p0 + dp * k + 4000, unfold_c), (p0 + dp * k + 5000, unfold_d)]
    merge(back, extra)
    for i in range(NT_):
        fin_out(i)
        fin_dx(i)
    for tw in late:
        run(tw)

    for cp in out_cp:
        cp.wait()


@jax.jit
def pallas_parallel_sum__linear_kernel_hedgehog__glu_gated_geglu__prompt_kernel(
    A_x: jax.Array,
    A_wqkv: jax.Array,
    A_w_phi: jax.Array,
    A_wo: jax.Array,
    B_x: jax.Array,
    B_w_gate: jax.Array,
    B_w_up: jax.Array,
    B_w_down: jax.Array,
    grad_out: jax.Array,
):
    del B_x
    xT = A_x.reshape(S, D).T
    dyT = grad_out.reshape(S, D).T
    wphi = A_w_phi.transpose(1, 0, 2).reshape(DH * H, DH)
    wdT = B_w_down.T

    vm = pltpu.VMEM
    sds = lambda *s: jax.ShapeDtypeStruct(s, BF16)
    out_shape = (sds(D, S), sds(D, S), sds(D, 3 * D), sds(D, DH), sds(D, D),
                 sds(D, DF), sds(D, DF), sds(D, DF))
    scratch = [
        vm((D, S), BF16), vm((D, S), BF16), vm((D, 3 * D), BF16), vm((D, DH), BF16),
        vm((D, D), BF16), vm((D, DF), BF16), vm((D, DF), BF16), vm((D, DF), BF16),
        vm((D, S), BF16), vm((2, NP, XF_W), BF16), vm((2, 7, DM, NP), BF16),
        vm((NG, GF, S), BF16), vm((NG, GE, S), BF16), vm((3 * D, S), BF16),
        vm((3 * D, D), BF16), vm((3 * D, D), BF16), vm((D, 3 * D), BF16), vm((D, D), BF16),
        vm((D, S), BF16), vm((D, S), BF16), vm((D, 3 * D), BF16), vm((D, DH), BF16),
        vm((D, D), BF16), vm((D, DF), BF16), vm((D, DF), BF16), vm((D, DF), BF16),
        pltpu.SemaphoreType.DMA((9,)), pltpu.SemaphoreType.DMA((23,)),
    ]
    any_spec = pl.BlockSpec(memory_space=pl.ANY)
    outT, dxT, dwqkv, dwphi, dwo, dwg, dwu, dwdT = pl.pallas_call(
        _kernel,
        out_shape=out_shape,
        in_specs=[any_spec] * 8,
        out_specs=[any_spec] * 8,
        scratch_shapes=scratch,
        compiler_params=pltpu.CompilerParams(vmem_limit_bytes=120 * 1024 * 1024),
    )(xT, dyT, A_wqkv, wphi, A_wo, B_w_gate, B_w_up, wdT)

    return (outT.T.reshape(1, S, D), dxT.T.reshape(1, S, D), dwqkv,
            dwphi.reshape(DH, H, DH).transpose(1, 0, 2), dwo, dwg, dwu, dwdT.T)
```

```python
import jax
import jax.numpy as jnp
import jax.experimental.pallas as pl
import jax.experimental.pallas.tpu as pltpu

F32 = jnp.float32
BF16 = jnp.bfloat16

S, D, H, DH, DF = 2048, 448, 16, 28, 1792
NG = H // 2
GR = 2 * DH
GE = 64
GF = 2 * GR
T = 512
TH = T // 2
NT_ = S // T
NP = S // 2
DA, DB = 256, 192
DM = D // 2
MB = 512
NM = NP // MB
CH = ((0, 256), (512, 256), (1024, 256), (1536, 128))
XF_W = 4 * DA + 9 * 128
LN_EPS = 1e-5
DEN_EPS = 1e-6
GELU_C1 = 0.7978845608028654
GELU_C2 = GELU_C1 * 0.044715
LOG2E = 1.4426950408889634


def _nn(a, b):
    return jnp.dot(a, b, preferred_element_type=F32)


def _nt(a, b):
    return jax.lax.dot_general(a, b, (((1,), (1,)), ((), ())),
                               preferred_element_type=F32)


def _iota(shape, dim):
    return jax.lax.broadcasted_iota(jnp.int32, shape, dim)


def _rows(*parts):
    return jnp.concatenate(parts, axis=0)


def _lanes(*parts):
    return jnp.concatenate(parts, axis=1)


def _seg_reduce(p, op, red, fill):
    low = _iota((p.shape[0], 8, p.shape[2]), 1) < 4
    v = [p[:, 8 * i:8 * i + 8, :] for i in range(7)]
    a = op(op(v[0], v[1]), op(v[2], jnp.where(low, v[3], fill)))
    b = op(op(v[4], v[5]), op(v[6], jnp.where(low, fill, v[3])))
    return red(a, axis=1, keepdims=True), red(b, axis=1, keepdims=True)


def _seg_mix(ra, rb):
    low = _iota((ra.shape[0], 8, ra.shape[2]), 1) < 4
    return jnp.where(low, ra, rb)


def _seg_sum(p):
    return _seg_reduce(p, jnp.add, jnp.sum, 0.0)


def _recip(x):
    r = pl.reciprocal(x, approx=True)
    return r * (2.0 - x * r)


def _pair_reduce(p, op):
    r = op(op(op(p[:, 0], p[:, 1]), op(p[:, 2], p[:, 3])), op(op(p[:, 4], p[:, 5]), p[:, 6]))
    r = op(r, pltpu.roll(r, 2, 1))
    r = op(r, pltpu.roll(r, 4, 1))
    return r[:, None]


def _softmax_pair(p):
    ep = jnp.exp2(p - _pair_reduce(p, jnp.maximum))
    en = jnp.exp2(_pair_reduce(p, jnp.minimum) - p)
    return ep * _recip(_pair_reduce(ep, jnp.add)), en * _recip(_pair_reduce(en, jnp.add))


def _softmax_pair_bwd(sp, sn, dsp, dsn):
    tp = sp * dsp
    tn = sn * dsn
    return (tp - sp * _pair_reduce(tp, jnp.add)) - (tn - sn * _pair_reduce(tn, jnp.add))


def _head_blocks(acc):
    r = _iota((NG, GE, GF), 1)
    c = _iota((NG, GE, GF), 2)
    row_b = ((r >= DH) & (r < GR)) | (r >= GR + 4)
    col_b = (c & 1) == 1
    m = jnp.where(row_b == col_b, acc, 0.0)
    padded = jnp.concatenate([m, jnp.zeros((NG, GE, 128 - GF), F32)], axis=2)
    z = padded.reshape(NG * GE, 128).T
    lane_lo = _iota((GF, 128), 1) < GE
    pairs = []
    for p in range(NG // 2):
        zp = z[:GF, 128 * p:128 * p + 128]
        pairs.append(jnp.concatenate(
            [jnp.where(lane_lo, zp, 0.0), jnp.where(lane_lo, 0.0, zp)], axis=0))
    return m.astype(BF16), jnp.stack(pairs).astype(BF16)


def _ffn_elem(g, u, dh):
    g2 = g * g
    t = jnp.tanh(g * (GELU_C1 + GELU_C2 * g2))
    a = 0.5 + 0.5 * t
    ge = g * a
    h = ge * u
    gp = a + ge * (1.0 - a) * (2.0 * GELU_C1 + (6.0 * GELU_C2) * g2)
    dg = dh * u * gp
    du = dh * ge
    return h, dg, du


_XS = (3, 4, 6)
_YS = (2, 4, 5)


def _zext(b, like, axis):
    n = like.shape[axis] - b.shape[axis]
    if n == 0:
        return b
    shape = (n, b.shape[1]) if axis == 0 else (b.shape[0], n)
    return jnp.concatenate([b, jnp.zeros(shape, b.dtype)], axis=axis)


def _head(op, a, b):
    n = b.shape[0]
    return op(a, b) if n == a.shape[0] else _rows(op(a[:n], b), a[n:])


def _bf(ops):
    return [o.astype(BF16) for o in ops]


def _x_ops(x, k):
    lo, hi = x[:, :TH], x[:, TH:]
    x11, x12, x21, x22 = lo[:k], lo[k:], hi[:k], hi[k:]
    return _bf([_head(jnp.add, x11, x22), _head(jnp.add, x21, x22), x11, x22,
                x11[:D - k] + x12, x21 - x11, x12 - x22])


def _w_ops(lo, hi, k):
    kh = hi.shape[1]
    w11, w12, w21, w22 = lo[:k], hi[:k], lo[k:], hi[k:]
    w22e = _zext(w22, w21, 1)
    return [_head(jnp.add, w11, w22e), w11, _head(jnp.subtract, w12, w22),
            w21 - w11[:D - k], w22, w11[:, :kh] + w12, w21 + w22e]


def _wt_ops(a):
    f = a.shape[0] // 2
    w11, w21, w12, w22 = a[:f, :DA], a[:f, DA:], a[f:, :DA], a[f:, DA:]
    w22e = _zext(w22, w11, 1)
    return [w11 + w22e, w11, w12 - w22e, w21 - w11[:, :DB], w22, w11 + w12, w21 + w22]


def _y_ops(y11, y12, y21, y22):
    return _bf([y11 + y22, y21 - y22, y12 + y22, y11 + y21, y12 - y11, y22, y11])


def _yt_ops(y11, y12, y21, y22):
    n = y12.shape[0]
    return _bf([_head(jnp.add, y11, y22), _head(jnp.subtract, y21, y22), y12 + y22,
                y11 + y21, y12 - y11[:n], y22, y11])


_Y_DONE = {3: 2, 4: 1, 5: 3, 6: 0}


def _y_block(n, p):
    if n == 3:
        return p(3) + p(1)
    if n == 4:
        return p(4) + p(2)
    if n == 5:
        return p(5) + p(0) - p(1) + p(2)
    return p(6) + p(0) + p(3) - p(4)


def _x_half(h, p):
    if h == 0:
        return _rows(p(4) + p(2) + p(0) - p(5), p(4) + p(6))
    return _rows(p(5) + p(1), p(0) + p(1) + p(3) - p(6))


def _w_from(p):
    return (p[1] + p[0] - p[3] + p[5], p[5] + p[2], p[6] + p[3],
            p[4] + p[0] - p[2] + p[6])


def _tri_left(a):
    return [a[0:128], a[64:192], _rows(a[0:64], a[128:192])]


def _tri_right(b):
    b1, b2 = b[:, :128], b[:, 128:]
    return [_rows(b1[0:64], b2[64:128]),
            _rows(b1[64:128] - b2[64:128], b1[128:192]),
            _rows(b2[0:64] - b1[0:64], b2[128:192])]


def _tri_rows(a):
    r = a.shape[0] // 2
    a1, a2 = a[:r], a[r:]
    d = a1[:, :128] - a2[:, :128]
    first = _iota((r, 128), 1) < 64
    return [jnp.where(first, a1[:, :128], a2[:, :128]),
            _lanes(a1[:, 128:], d[:, 64:]),
            _lanes(-d[:, :64], a2[:, 128:])]


_TRI_K = ((0, 64), (128, 64), (0, 128))

_XF_OFF = {0: 0, 1: DA, 2: 2 * DA, 5: 3 * DA,
           3: 4 * DA, 4: 4 * DA + 384, 6: 4 * DA + 768}
GU = ("g", "u")
PQ, PV, PX = 208, 224, 32
PK = 2 * PQ + PV
PL = PK + 2 * PX
_P_OFF = (0, PQ, 2 * PQ)

RATE = 2.0
BACKLOG = 200
LAT = 150
N_EARLY = 5
T_FFN = 250000
T_ATT = 235000
T_FIN = 265000


class _Task:
    def __init__(self, name, d, ops, deps, fn, at=0, fence=False):
        self.name, self.d, self.v, self.deps, self.fn = name, d, ops / RATE, deps, fn
        self.at, self.fence, self.due = at, fence, 0


def _order(tasks):
    pending = sorted(tasks, key=lambda x: x.due)
    done, t, vq, seq = {}, 0.0, 0.0, []
    while pending:
        cand = [(max([x.at] + [done[d] for d in x.deps]), x) for x in pending
                if all(d in done for d in x.deps)]
        ready = [x for r, x in cand if r <= t]
        light = [x for x in ready if x.v <= x.d / 2 and not x.fence]
        if ready and (vq - t <= BACKLOG or not light):
            pick = ready[0]
        elif ready:
            pick = light[0]
        else:
            t, pick = min(cand, key=lambda e: e[0])
        pending.remove(pick)
        seq.append((t, pick))
        if pick.fence:
            t = max(t, vq)
        vq = max(vq, t) + pick.v
        t += pick.d
        done[pick.name] = (max(t, vq) if pick.v > pick.d / 2 else t) + LAT
        done["order", pick.name] = 0
    return seq


def _kernel(xT_h, dyT_h, wqkv_h, wphi_h, wo_h, wg_h, wu_h, wdT_h,
            outT_h, dxT_h, dwqkv_h, dwphi_h, dwo_h, dwg_h, dwu_h, dwdT_h,
            xT, dyT, wqkv, wphi, wo, wg, wu, wdT,
            xnT, xf_s, xb_s, xw_s, phi_s, vext_s, yo_s, yp_s, wqkvT,
            sem_in, sem_out):
    outT, dxT, dwqkv, dwphi, dwo, dwg, dwu, dwdT = xT, dyT, wqkv, wphi, wo, wg, wu, wdT
    cols = lambda i: slice(i * T, (i + 1) * T)
    prs = lambda i: slice(i * TH, (i + 1) * TH)
    blk = lambda m: slice(m * MB, (m + 1) * MB)

    in_list = [
        ("wphi", wphi_h, wphi),
        ("wo", wo_h, wo),
        ("dy0", dyT_h.at[:, cols(0)], dyT.at[:, cols(0)]),
        ("dy1", dyT_h.at[:, T:], dyT.at[:, T:]),
        ("wd", wdT_h, wdT),
        ("x", xT_h, xT),
        ("wqkv", wqkv_h, wqkv),
        ("wg", wg_h, wg),
        ("wu", wu_h, wu),
    ]
    in_cp = {}
    for n, (name, h, v) in enumerate(in_list):
        in_cp[name] = pltpu.make_async_copy(h, v, sem_in.at[n])
        in_cp[name].start()
    out_cp = []

    def send(src, dst):
        cp = pltpu.make_async_copy(src, dst, sem_out.at[len(out_cp)])
        cp.start()
        out_cp.append(cp)

    V = {}

    def acc(key, val):
        V[key] = val + V[key] if key in V else val

    def wait(*names):
        for n in names:
            in_cp[n].wait()

    def rounds(name, rows, ops, deps, jobs):
        out = []
        for k in range(0, len(jobs), 4):
            js = jobs[k:k + 4]
            last = k + 4 >= len(jobs)
            out.append(_Task(name if last else (name, k), rows, ops * 4 / len(jobs),
                             deps if k == 0 else [("order", out[-1].name)],
                             lambda js=js: [j() for j in js]))
        return out

    def tri_jobs(lhs, rhs, put):
        st = {}

        def j0():
            st[0] = _nn(lhs(0), rhs(0))

        def j1():
            st[1] = _nn(lhs(1), rhs(1)) + st[0]

        def j2():
            put(st[1], _nn(lhs(2), rhs(2)) + st[0])
        return [j0, j1, j2]

    def tri_rhs(ref, idx, r0, lanes):
        return lambda k: _rows(*[ref[(*idx, slice(r0 + o, r0 + o + 64), lanes)] for o in _TRI_K[k]])

    def prep_x(which, i, x):
        for n, op in enumerate(_x_ops(x, DA)):
            xb_s[which, n, :op.shape[0], prs(i)] = op
            off = _XF_OFF[n]
            for pc in (_tri_left(op) if n in _XS else [op]):
                xf_s[which, prs(i), off:off + pc.shape[0]] = pc.T
                off += pc.shape[0]
        for n, op in enumerate(_x_ops(x, DM)):
            xw_s[which, n, :, prs(i)] = op

    def prep_w(name, ref, c):
        c0, w = CH[c]
        lo = ref[:, c0:c0 + w].astype(F32)
        hi = ref[:, c0 + w:c0 + 2 * w].astype(F32)
        fw = []
        for n, op in enumerate(_w_ops(lo, hi, DA)):
            if n not in _XS:
                fw.append(_bf([op]))
            elif w == 256:
                fw.append(_bf(_tri_right(op)))
            else:
                fw.append(_bf([_rows(op[:128], jnp.zeros((64, w), F32), op[128:])]))
        V["wf", name, c] = fw
        V["wr", name, c] = _bf(_w_ops(lo, hi, DM))

    def prep_t(name, a):
        V["wt", name] = [_bf(_tri_rows(op) if n in _XS else [op])
                         for n, op in enumerate(_wt_ops(a))]

    RQ = MB // 4

    def f_put(nm, c, m, n, r0, val):
        for r in range(0, val.shape[0], RQ):
            q = (r0 + r) // RQ
            V["p", nm, c, m, n, q] = val[r:r + RQ]
            if n in _Y_DONE:
                V["y", nm, c, m, _Y_DONE[n], q] = _y_block(n, lambda k: V["p", nm, c, m, k, q])
                if nm == "u":
                    f_elem(c, m, _Y_DONE[n], q)

    def f_elem(c, m, b, q):
        V["e", c, m, b, q] = _ffn_elem(*[V.pop(("y", nm, c, m, b, q)) for nm in ("g", "u", "d")])
        if b == 0:
            h, dg, du = zip(*[V.pop(("e", c, m, bb, q)) for bb in range(4)])
            V["z", 1, c, m, q] = _y_ops(*h)
            V["z", 0, c, m, q] = [_lanes(a, b_) for a, b_ in zip(_y_ops(*dg), _y_ops(*du))]

    def f_long(names, c, m, n, r0, rn):
        which, w, off = int(names[0] == "d"), CH[c][1], _XF_OFF[n]
        p = _nn(xf_s[which, m * MB + r0:m * MB + r0 + rn, off:off + DA],
                _lanes(*[V["wf", nm, c][n][0] for nm in names]))
        for k, nm in enumerate(names):
            f_put(nm, c, m, n, r0, p[:, k * w:(k + 1) * w])

    def f_tri(nm, c, m, n, q):
        which, off, r0 = int(nm == "d"), _XF_OFF[n], m * MB + q * RQ
        return tri_jobs(lambda k: xf_s[which, r0:r0 + RQ, off + 128 * k:off + 128 * k + 128],
                        lambda k: V["wf", nm, c][n][k],
                        lambda c1, c2: f_put(nm, c, m, n, q * RQ, _lanes(c1, c2)))

    def t_fd(c):
        out = []
        for m in range(NM):
            for n in range(7):
                deps = [("pw", "d", c), ("px", 1, 2 * m), ("px", 1, 2 * m + 1)]
                if n:
                    deps.append(("order", ("fd", c, m, n - 1)))
                name = ("fd", c, m, n)
                if CH[c][1] == 128:
                    out.append(_Task(name, MB // 2, 0, deps, lambda m=m, n=n: [
                        f_long(("d",), c, m, n, r0, MB // 2) for r0 in (0, MB // 2)]))
                elif n in _XS:
                    jobs = [j for q in range(4) for j in f_tri("d", c, m, n, q)]
                    out.append(_Task(name, 3 * RQ, 0, deps, lambda jobs=jobs: [j() for j in jobs]))
                else:
                    out.append(_Task(name, MB, 0, deps,
                                     lambda m=m, n=n: f_long(("d",), c, m, n, 0, MB)))
        return out

    def t_fgu(c, m):
        w = CH[c][1]
        deps = [("pw", "gu", c), ("px", 0, 2 * m), ("px", 0, 2 * m + 1)]
        out = []
        for n in range(3):
            for names in ([GU] if w == 128 else [("g",), ("u",)]):
                out.append(_Task(("fp", c, m, n, names[-1]), MB, 0, deps,
                                 lambda n=n, names=names: f_long(names, c, m, n, 0, MB)))
        prev = [("order", t.name) for t in out] + [("order", ("fd", c, m, 6))]
        gelu = 30 * (RQ // 8) * (w // 128)
        for q2 in (0, 2):
            for n in range(3, 7):
                name = ("fc", c, m, n, q2)
                if w == 256 and n in _XS:
                    jobs = [j for q in (q2, q2 + 1) for nm in GU for j in f_tri(nm, c, m, n, q)]
                    out += rounds(name, RQ, 2 * gelu, prev, jobs)
                else:
                    parts = [(q, names) for q in (q2, q2 + 1)
                             for names in ([GU] if w == 128 else [("g",), ("u",)])]
                    for k, (q, names) in enumerate(parts):
                        out.append(_Task(name if k + 1 == len(parts) else (name, k), RQ,
                                         2 * gelu / len(parts), prev,
                                         lambda n=n, q=q, names=names: f_long(names, c, m, n, q * RQ, RQ)))
                        prev = [("order", out[-1].name)]
                prev = [("order", out[-1].name)]
        return out

    def z_op(which, c, m, n):
        return _rows(*[V["z", which, c, m, q][n] for q in range(4)])

    def acc_x(which, m, n, val, l0=0):
        for l in range(0, val.shape[1], 128):
            acc(("ax", which, m, n, (l0 + l) // 128), val[:, l:l + 128])

    def bwd_x(which, c, m, n):
        lhs = _lanes(*[V["wr", nm, c][n] for nm in (("d",) if which else GU)])
        acc_x(which, m, n, _nt(lhs, z_op(which, c, m, n)))

    def bwd_w(which, c, m, n):
        acc(("aw", which, c, n), _nn(xw_s[which, n, :, blk(m)], z_op(which, c, m, n)))

    def fin_w(which, c):
        c0, w = CH[c]
        q = _w_from([V.pop(("aw", which, c, n)) for n in range(7)])
        refs = ((dwg, dwg_h), (dwu, dwu_h)) if which == 0 else ((dwdT, dwdT_h),)
        for k, (ref, hbm) in enumerate(refs):
            sl = slice(k * w, (k + 1) * w)
            ref[:DM, c0:c0 + w] = q[0][:, sl].astype(BF16)
            ref[:DM, c0 + w:c0 + 2 * w] = q[1][:, sl].astype(BF16)
            ref[DM:, c0:c0 + w] = q[2][:, sl].astype(BF16)
            ref[DM:, c0 + w:c0 + 2 * w] = q[3][:, sl].astype(BF16)
            send(ref.at[:, c0:c0 + 2 * w], hbm.at[:, c0:c0 + 2 * w])

    W_ORD = (0, 2, 3, 5, 6, 1, 4)
    X_ORD = (1, 3, 0, 6, 5, 2, 4)

    def t_bx(c, m):
        d = DM * CH[c][1] // 128
        return [_Task(("bx", which, c, m, n), d * (2 - which), 0, [("fc", c, m, 6, 2)],
                      lambda which=which, n=n: bwd_x(which, c, m, n))
                for which in (1, 0) for n in X_ORD]

    def t_bw(which, c, m):
        d = DM * CH[c][1] // 128 * (2 - which)
        out = []
        for n in W_ORD:
            deps = [("fc", c, m, 6, 2)] + ([("order", ("bw", which, c, m - 1, n))] if m else [])
            out.append(_Task(("bw", which, c, m, n), d, 0, deps,
                             lambda n=n: bwd_w(which, c, m, n)))
        if m == NM - 1:
            out.append(_Task(("fw", which, c), 0, 0, [("order", t.name) for t in out],
                             lambda: fin_w(which, c)))
        return out

    def consts():
        r = _iota((D, D), 0)
        c = _iota((D, D), 1)
        V["perm"] = jnp.where(r == (c & 15) * DH + (c >> 4), 1.0, 0.0).astype(BF16)
        V["perm_t"] = jnp.where(c == (r & 15) * DH + (r >> 4), 1.0, 0.0).astype(BF16)
        rr = _iota((GF, DH), 0)
        rc = _iota((GF, DH), 1)
        V["rep"] = jnp.where((rr >> 1 == rc) | (rr >> 1 == rc + DH), 1.0, 0.0).astype(BF16)
        br = _iota((GF, GF), 0)
        bc = _iota((GF, GF), 1)
        hd = lambda t: ((t >= DH).astype(jnp.int32) + (t >= 2 * DH).astype(jnp.int32)
                        + (t >= 3 * DH).astype(jnp.int32))
        hf = lambda t: 2 * (t >= GR).astype(jnp.int32) + (t & 1)
        V["diag_t"] = jnp.where(hf(br) == hd(bc), 1.0, 0.0)
        V["diag"] = jnp.where(hd(br) == hf(bc), 1.0, 0.0)

    def phi_a():
        V["wphi_hd"] = _nn(V["perm"], wphi[...]).astype(BF16)

    def phi_b():
        whd, rep, diag = V["wphi_hd"], V["rep"], V["diag"] > 0.5
        V["phi_t"] = [jnp.where(V["diag_t"] > 0.5, _nt(rep, whd[GF * g:GF * g + GF]), 0.0).astype(BF16)
                      for g in range(4)]
        V["phi_n"] = [jnp.where(diag, _nt(whd[GF * g:GF * g + GF], rep), 0.0).astype(BF16)
                      for g in range(4)]

    def prep_wo():
        prep_t("o", wo[...].astype(F32))
        woT = wo[...].T.astype(F32)
        V["wa"] = [_bf(_tri_rows(op) if n in _YS else [op])
                   for n, op in enumerate(_w_ops(woT[:, :DA], woT[:, DA:], DM))]

    def tr_qkv():
        wqkvT[...] = wqkv[...].T

    def fold(t):
        if t < 2:
            V["WT", t] = _rows(*[_nn(V["phi_t"][g], wqkvT[D * t + GF * g:D * t + GF * g + GF, :])
                                 for g in range(4)])
        else:
            V["WT", t] = wqkvT[2 * D:, :].astype(F32)
        prep_t(t, V["WT", t] * LOG2E if t < 2 else V["WT", t])

    def prep_wp():
        q, k, v = [V.pop(("WT", t)) for t in range(3)]
        lo = _rows(q[:PQ], k[:PQ], v[:PV], q[2 * PQ:], k[2 * PQ:]).T
        hi = _rows(q[PQ:2 * PQ], k[PQ:2 * PQ], v[PV:]).T
        V["wp"] = [_bf([op] if n in _YS else [op[:, :PL - DB]] + _tri_rows(op[:, PL - DB:]))
                   for n, op in enumerate(_w_ops(lo, hi, DM))]

    def ln(i):
        x = xT[:, cols(i)].astype(F32)
        xc = x - jnp.mean(x, axis=0, keepdims=True)
        rstd = jax.lax.rsqrt(jnp.mean(xc * xc, axis=0, keepdims=True) + LN_EPS)
        xn = xc * rstd
        V["rstd", i] = rstd
        xnT[:, cols(i)] = xn.astype(BF16)
        prep_x(0, i, xn)

    def a_sink(t, f, c0, y):
        w = y.shape[1]
        gs, cs = slice(4 * f, 4 * f + 4), slice(c0, c0 + w)
        if t == "o":
            for l in range(0, w, 128):
                V["do", f, c0 + l] = y[:, l:l + 128]
        elif t == 2:
            vext_s[gs, :, cs] = jnp.concatenate(
                [y.reshape(4, GR, w), jnp.ones((4, 8, w), F32)], axis=1).astype(BF16)
        else:
            phi_s[t, gs, :, cs] = jnp.concatenate(
                _softmax_pair(y.reshape(4, 7, 8, w)), axis=1).reshape(4, GF, w).astype(BF16)

    def a_put(t, m, n, l0, val):
        for l in range(0, val.shape[1], 128):
            k = (l0 + l) // 128
            V["ap", t, m, n, k] = val[:, l:l + 128]
            if n in _Y_DONE:
                h, f = divmod(_Y_DONE[n], 2)
                a_sink(t, f, (2 * m + k // 2) * T + h * TH + (k % 2) * 128,
                       _y_block(n, lambda j: V["ap", t, m, j, k]))

    def t_proj(t, m):
        which = int(t == "o")
        deps = [("pt", t), ("px", which, 2 * m), ("px", which, 2 * m + 1)]
        ops = 16 * 100 if t in (0, 1) else 0
        out = []
        for n in range(7):
            name = ("ap", t, m, n)
            if n in _XS:
                jobs = [j for k in range(4) for j in tri_jobs(
                    lambda s, n=n: V["wt", t][n][s],
                    tri_rhs(xb_s, (which, n), 0, slice(m * MB + 128 * k, m * MB + 128 * k + 128)),
                    lambda c1, c2, n=n, k=k: a_put(t, m, n, 128 * k, _rows(c1, c2)))]
                out += rounds(name, DM // 2, ops, deps, jobs)
            else:
                for l0 in (0, TH):
                    out.append(_Task(
                        name if l0 else (name, 0), DM, ops / 2 if n in _Y_DONE else 0, deps,
                        lambda n=n, l0=l0: a_put(t, m, n, l0, _nn(
                            V["wt", t][n][0], xb_s[which, n, :, m * MB + l0:m * MB + l0 + TH]))))
                    deps = [("order", out[-1].name)]
            deps = [("order", out[-1].name)]
        return out

    def do_plain(i):
        p = _nn(wo[...], dyT[:, cols(i)])
        for f in range(2):
            a_sink("o", f, i * T, p[DM * f:DM * f + DM])

    def k_state(i, p):
        for j in (2 * p, 2 * p + 1):
            acc(("kv", j), _nt(vext_s[j, :, cols(i)], phi_s[1, j, :, cols(i)]))

    def blocks(name):
        V[name, "T"], V[name, "P"] = _head_blocks(jnp.stack([V.pop((name, j)) for j in range(NG)]))

    def q_mid(i, p):
        low = _iota((2, 8, T), 1) < 4
        ne = jnp.stack([_nn(V["kv", "T"][j], phi_s[0, j, :, cols(i)]) for j in (2 * p, 2 * p + 1)])
        rmix = _recip(ne[:, GR:, :] + DEN_EPS)
        rrot = pltpu.roll(rmix, 4, 1)
        ra = jnp.where(low, rmix, rrot)
        rb = jnp.where(low, rrot, rmix)
        rden = jnp.concatenate([ra, ra, ra, rmix, rb, rb, rb], axis=1)
        o = ne[:, :GR, :] * rden
        r0 = GF * (p % 2)
        do = _lanes(*[V["do", p // 2, i * T + l][r0:r0 + GF] for l in range(0, T, 128)])
        dnum = do.reshape(2, GR, T) * rden
        dden = _seg_mix(*_seg_sum(dnum * o)) * (-0.25)
        V["dne", i, p] = jnp.concatenate([dnum, dden], axis=1).astype(BF16)
        V["o", i, p] = o.reshape(GF, T)
        if p == 3:
            o = _rows(*[V.pop(("o", i, s)) for s in range(4)])
            for n, op in enumerate(_yt_ops(o[:DA, :TH], o[DA:, :TH], o[:DA, TH:], o[DA:, TH:])):
                yo_s[n, :op.shape[0], prs(i)] = op

    def dp_put(t, i, p, val):
        V["dp", t, i, p] = val
        if p < 3:
            return
        y = _rows(*[V.pop(("dp", t, i, s)) for s in range(4)])
        r, off = (PV if t == 2 else PQ), _P_OFF[t]
        for n, op in enumerate(_y_ops(y[:r, :TH], y[r:2 * r, :TH], y[:r, TH:], y[r:2 * r, TH:])):
            yp_s[n, off:off + r, prs(i)] = op
        if t < 2:
            lo, hi = y[2 * r:, :TH], y[2 * r:, TH:]
            for n, op in zip((0, 1, 3, 6), _bf([lo, hi, lo + hi, lo])):
                yp_s[n, PK + PX * t:PK + PX * t + PX, prs(i)] = op

    def phi_bwd(t, i, p):
        if t == 0:
            dphi = _nn(V["kv", "P"][p], V["dne", i, p].reshape(2 * GE, T))
        else:
            dphi = _nn(V["dkv", "P"][p], vext_s[2 * p:2 * p + 2, :, cols(i)].reshape(2 * GE, T))
        dphi = dphi.reshape(2, 14, 8, T)
        pf = phi_s[t, 2 * p:2 * p + 2, :, cols(i)].astype(F32).reshape(2, 14, 8, T)
        dp = _softmax_pair_bwd(pf[:, :7], pf[:, 7:], dphi[:, :7], dphi[:, 7:])
        dp_put(t, i, p, dp.reshape(GF, T))

    def q_state(i, p):
        dne = V["dne", i, p]
        for s in range(2):
            acc(("dkv", 2 * p + s), _nt(dne[s], phi_s[0, 2 * p + s, :, cols(i)]))

    def dv_mm(i, p):
        dp_put(2, i, p, _rows(*[_nn(V["dkv", "T"][j], phi_s[1, j, :, cols(i)])[:GR]
                                for j in (2 * p, 2 * p + 1)]))

    def x_tri(name, which, wname, ref, r0, m, n, deps):
        jobs = [j for k in range(4) for j in tri_jobs(
            lambda s: V[wname][n][s - 3],
            tri_rhs(ref, (n,), r0, slice(m * MB + 128 * k, m * MB + 128 * k + 128)),
            lambda c1, c2, k=k: acc_x(which, m, n, _rows(c1, c2), 128 * k))]
        return _Task(name, 3 * DM // 2, 0, deps, lambda: [j() for j in jobs])

    def t_outa(m):
        deps = [("qm", 2 * m, 3), ("qm", 2 * m + 1, 3), "pwo"]
        return [x_tri(("oa", m, n), 1, "wa", yo_s, 0, m, n, deps) if n in _YS else
                _Task(("oa", m, n), 2 * DM, 0, deps,
                      lambda n=n: acc_x(1, m, n, _nn(V["wa"][n][0], yo_s[n, :, blk(m)])))
                for n in X_ORD]

    def dwo_mm(m, n):
        acc(("ao", n), _nt(yo_s[n, :DB if n in _YS else DA, blk(m)],
                           xb_s[1, n, :DB if n in _XS else DA, blk(m)]))

    def fin_wo():
        p = [V.pop(("ao", n)) for n in range(7)]
        dwo[:DA, :DA] = _head(jnp.add, p[1] + p[0] - _zext(p[3], p[0], 1), p[5]).astype(BF16)
        dwo[DA:, :DA] = (p[5] + p[2]).astype(BF16)
        dwo[:DA, DA:] = (p[6] + p[3]).astype(BF16)
        dwo[DA:, DA:] = (p[4] + p[0][:DB, :DB] - p[2][:, :DB] + p[6][:DB]).astype(BF16)
        send(dwo, dwo_h)

    def t_dwo(m):
        out = [_Task(("ao", m, n), 2 * (DB if n in _YS else DA), 0,
                     [("qm", 2 * m, 3), ("qm", 2 * m + 1, 3)]
                     + ([("order", ("ao", m - 1, n))] if m else []),
                     lambda n=n: dwo_mm(m, n)) for n in W_ORD]
        if m == NM - 1:
            out.append(_Task("fwo", 0, 0, [("order", t.name) for t in out], fin_wo))
        return out

    def dp_deps(m):
        return [(s, i, 3) for s in ("qb", "kb", "dv") for i in (2 * m, 2 * m + 1)]

    def t_dxn(m, extra):
        out = []
        for n in X_ORD:
            deps = dp_deps(m) + ["pwp"]
            if n in _YS:
                deps = deps + extra + [("order", t.name) for t in out]
                jobs = [lambda k=k, s=s, n=n: acc_x(0, m, n, _nn(
                    V["wp"][n][0][:, 128 * s:128 * s + 128],
                    yp_s[n, 128 * s:128 * s + 128, m * MB + 128 * k:m * MB + 128 * k + 128]), 128 * k)
                    for k in range(4) for s in range(5)]
                out += rounds(("dx", m, n), DM, 0 if n == 2 else 224 * 12, deps, jobs)
                if n != 2:
                    out.append(_Task(("fdx", m, n), 0, 0, [("order", out[-1].name)],
                                     lambda n=n: fin_dx(m, int(n == 5))))
            else:
                out.append(_Task(("dx", m, n, 0), 4 * DM, 0, deps, lambda n=n: acc_x(
                    0, m, n, _nn(V["wp"][n][0], yp_s[n, :PL - DB, blk(m)]))))
                out.append(x_tri(("dx", m, n), 0, "wp", yp_s, PL - DB, m, n, deps))
        return out

    def g_mm(m, n):
        acc(("ag", n), _nt(xw_s[0, n, :, blk(m)], yp_s[n, :PK, blk(m)]))

    def gx_mm(i):
        acc("gx", _nt(_lanes(yp_s[0, PK:, prs(i)], yp_s[1, PK:, prs(i)]), xnT[:, cols(i)]))

    def t_g(m):
        out = [_Task(("gx", i), 4 * GE, 0, dp_deps(m), lambda i=i: gx_mm(i))
               for i in (2 * m, 2 * m + 1)]
        out += [_Task(("ag", m, n), 5 * DM, 0,
                      dp_deps(m) + ([("order", ("ag", m - 1, n))] if m else []),
                      lambda n=n: g_mm(m, n)) for n in W_ORD]
        return out

    def x_cols(which, m, h, i):
        k0 = 2 * (i - 2 * m)
        return _x_half(h, lambda n: _lanes(V["ax", which, m, n, k0], V["ax", which, m, n, k0 + 1]))

    def fin_out(m):
        for i in (2 * m, 2 * m + 1):
            for h in range(2):
                cs = slice(i * T + h * TH, i * T + h * TH + TH)
                outT[:, cs] = (x_cols(1, m, h, i) + xT[:, cs].astype(F32)).astype(BF16)
            send(outT.at[:, cols(i)], outT_h.at[:, cols(i)])

    def fin_dx(m, h):
        for i in (2 * m, 2 * m + 1):
            cs = slice(i * T + h * TH, i * T + h * TH + TH)
            dxn = x_cols(0, m, h, i)
            xf = xnT[:, cs].astype(F32)
            m1 = jnp.mean(dxn, axis=0, keepdims=True)
            m2 = jnp.mean(dxn * xf, axis=0, keepdims=True)
            dxT[:, cs] = (dyT[:, cs].astype(F32)
                          + (dxn - m1 - xf * m2) * V["rstd", i][:, h * TH:h * TH + TH]).astype(BF16)
            send(dxT.at[:, cs], dxT_h.at[:, cs])

    def unfold_a():
        w11, w12, w21, w22 = _w_from([V.pop(("ag", n)) for n in range(7)])
        lo = _rows(w11, w21).astype(BF16).T
        hi = _rows(w12, w22).astype(BF16).T
        gx = V.pop("gx").astype(BF16)
        V["gT"] = _rows(lo[:PQ], hi[:PQ], gx[:PX], lo[PQ:2 * PQ], hi[PQ:2 * PQ], gx[PX:],
                        lo[2 * PQ:], hi[2 * PQ:])

    def unfold_b():
        gT = V["gT"]
        dwT = _rows(*[_nn(V["phi_n"][g % 4], gT[GF * g:GF * g + GF]).astype(BF16)
                      for g in range(8)], gT[2 * D:])
        dwqkv[...] = dwT.T
        send(dwqkv, dwqkv_h)

    def unfold_c():
        gT = V["gT"]
        diag = V["diag"] > 0.5
        V["xqk"] = []
        for g in range(4):
            xq = _nt(wqkvT[GF * g:GF * g + GF, :], gT[GF * g:GF * g + GF])
            xk = _nt(wqkvT[D + GF * g:D + GF * g + GF, :], gT[D + GF * g:D + GF * g + GF]) + xq
            V["xqk"].append(jnp.where(diag, xk, 0.0).astype(BF16))

    def unfold_d():
        V["ys"] = _rows(*[_nn(t, V["rep"]).astype(BF16) for t in V.pop("xqk")])

    def unfold_e():
        dwphi[...] = _nn(V["perm_t"], V.pop("ys")).astype(BF16)
        send(dwphi, dwphi_h)

    def spread(tasks, t0, t1):
        tot, pos = sum(x.d for x in tasks), 0
        for x in tasks:
            x.due = t0 + (t1 - t0) * pos / max(tot, 1)
            pos += x.d
        return tasks

    nc = len(CH)
    px_dy = lambda i: _Task(("px", 1, i), 0, 1500, ["w1" if i == 0 else "w2"],
                            lambda: prep_x(1, i, dyT[:, cols(i)].astype(F32)))
    start = [
        _Task("w1", 0, 0, [], lambda: wait("wphi", "wo", "dy0"), fence=True),
        _Task("phi_a", D, 0, ["w1"], phi_a),
        _Task(("do", 0), 4 * D, 0, ["w1"], lambda: do_plain(0)),
        px_dy(0),
        _Task("phi_b", 2 * GF, 0, ["phi_a"], phi_b),
        _Task("w2", 0, 0, [("order", "phi_b"), ("order", ("do", 0))], lambda: wait("dy1"), fence=True),
        _Task(("do", 1), 4 * D, 0, ["w2"], lambda: do_plain(1)),
        _Task("pwo", 0, 1500, ["w2"], prep_wo),
        _Task(("pt", "o"), 0, 0, ["pwo"], lambda: None),
        px_dy(2), px_dy(3), px_dy(1),
    ] + t_proj("o", 1) + [
        _Task("w3", 0, 0, [("order", ("ap", "o", 1, 6))], lambda: wait("wd"), fence=True)]
    for c in range(nc):
        start.append(_Task(("pw", "d", c), 0, 1200, ["w3"], lambda c=c: prep_w("d", wdT, c)))
        start += t_fd(c)
        if c == 1:
            start.append(_Task("w4", 0, 0, [("order", start[-1].name)],
                               lambda: wait("x", "wqkv", "wg", "wu"), fence=True))
    spread(start, 0, 30000)

    prep = [_Task("trq", 0, 600, ["w4"], tr_qkv),
            _Task(("px", 0, 0), 0, 3000, ["w4"], lambda: ln(0)),
            _Task(("pt", 1), D, 1000, ["trq", "phi_b"], lambda: fold(1)),
            _Task(("px", 0, 1), 0, 3000, ["w4"], lambda: ln(1)),
            _Task(("pt", 2), 0, 1000, ["trq"], lambda: fold(2)),
            _Task(("pt", 0), D, 1000, ["trq", "phi_b"], lambda: fold(0)),
            _Task(("px", 0, 2), 0, 3000, ["w4"], lambda: ln(2)),
            _Task(("px", 0, 3), 0, 3000, ["w4"], lambda: ln(3))]
    for k, x in enumerate(prep):
        x.due = 19000 + k

    steps = [(c, m) for c in range(nc) for m in range(NM)]
    ffn, late = [], []
    for k, (c, m) in enumerate(steps + [(None, None)]):
        if c is not None:
            if m == 0:
                ffn.append(_Task(("pw", "gu", c), 0, 2400, ["w4"],
                                 lambda c=c: (prep_w("g", wg, c), prep_w("u", wu, c))))
            ffn += t_fgu(c, m)
        if k:
            c, m = steps[k - 1]
            ffn += t_bx(c, m)
            (ffn if k - 1 < N_EARLY else late).extend(t_bw(0, c, m) + t_bw(1, c, m))
    spread(ffn, 30000, T_FFN)

    att = []
    q4 = range(4)
    for m in range(NM):
        att += t_proj(1, m) + t_proj(2, m)
        att += [_Task(("ks", i, p), 2 * GE, 0, [("ap", 1, m, 6), ("ap", 2, m, 6)],
                      lambda i=i, p=p: k_state(i, p)) for i in (2 * m, 2 * m + 1) for p in q4]
    att.append(_Task("kv", 0, 600, [("ks", i, p) for i in q4 for p in q4], lambda: blocks("kv")))
    att.append(_Task("pwp", 0, 3000, [("pt", t) for t in range(3)], prep_wp))
    for m in range(NM):
        att += t_proj(0, m)
        for i in (2 * m, 2 * m + 1):
            att += [_Task(("qm", i, p), 2 * GE, 520,
                          ["kv", ("ap", 0, m, 6)] + ([("order", ("qm", i, p - 1))] if p else []),
                          lambda i=i, p=p: q_mid(i, p)) for p in q4]
            att += [_Task(("qs", i, p), 2 * GE, 0, [("qm", i, p)], lambda i=i, p=p: q_state(i, p))
                    for p in q4]
            att += [_Task(("qb", i, p), DM, 900,
                          [("qm", i, p)] + ([("order", ("qb", i, p - 1))] if p else []),
                          lambda i=i, p=p: phi_bwd(0, i, p)) for p in q4]
        att += t_outa(m) + t_dwo(m)
    att.append(_Task("dkv", 0, 600, [("qs", i, p) for i in q4 for p in q4], lambda: blocks("dkv")))
    for m in range(NM):
        for i in (2 * m, 2 * m + 1):
            for p in q4:
                att.append(_Task(("kb", i, p), DM, 900,
                                 ["dkv"] + ([("order", ("kb", i, p - 1))] if p else []),
                                 lambda i=i, p=p: phi_bwd(1, i, p)))
                att.append(_Task(("dv", i, p), 2 * GE, 130,
                                 ["dkv"] + ([("order", ("dv", i, p - 1))] if p else []),
                                 lambda i=i, p=p: dv_mm(i, p)))
        att += t_g(m)
    att += [_Task("ua", 0, 2000, [("ag", NM - 1, n) for n in range(7)] + [("gx", i) for i in q4],
                  unfold_a),
            _Task("ub", 8 * GF, 0, ["ua"], unfold_b),
            _Task("uc", 8 * GF, 0, ["ua"], unfold_c),
            _Task("ud", GF, 0, ["uc"], unfold_d),
            _Task("ue", D, 0, ["ud"], unfold_e)]
    spread(att, 31000, T_ATT)

    fin = []
    for m in range(NM):
        fin.append(_Task(("fo", m), 0, 2000,
                         [("order", ("bx", 1, c, m, n)) for c in range(nc) for n in range(7)]
                         + [("order", ("oa", m, n)) for n in range(7)], lambda m=m: fin_out(m)))
        fin += t_dxn(m, [("order", ("bx", 0, c, m, n)) for c in range(nc) for n in range(7)])
    spread(fin, T_ATT, T_FIN)
    spread(late, T_FIN, T_FIN + 20000)

    consts()
    for _, x in _order(start + prep + ffn + att + fin + late):
        x.fn()
    for cp in out_cp:
        cp.wait()


@jax.jit
def pallas_parallel_sum__linear_kernel_hedgehog__glu_gated_geglu__prompt_kernel(
    A_x: jax.Array,
    A_wqkv: jax.Array,
    A_w_phi: jax.Array,
    A_wo: jax.Array,
    B_x: jax.Array,
    B_w_gate: jax.Array,
    B_w_up: jax.Array,
    B_w_down: jax.Array,
    grad_out: jax.Array,
):
    del B_x
    xT = A_x.reshape(S, D).T
    dyT = grad_out.reshape(S, D).T
    wphi = A_w_phi.transpose(1, 0, 2).reshape(DH * H, DH)
    wdT = B_w_down.T

    vm = pltpu.VMEM
    sds = lambda *s: jax.ShapeDtypeStruct(s, BF16)
    out_shape = (sds(D, S), sds(D, S), sds(D, 3 * D), sds(D, DH), sds(D, D),
                 sds(D, DF), sds(D, DF), sds(D, DF))
    scratch = [
        vm((D, S), BF16), vm((D, S), BF16), vm((D, 3 * D), BF16), vm((D, DH), BF16),
        vm((D, D), BF16), vm((D, DF), BF16), vm((D, DF), BF16), vm((D, DF), BF16),
        vm((D, S), BF16), vm((2, NP, XF_W), BF16), vm((2, 7, DA, NP), BF16),
        vm((2, 7, DM, NP), BF16), vm((2, NG, GF, S), BF16), vm((NG, GE, S), BF16),
        vm((7, DA, NP), BF16), vm((7, PL, NP), BF16), vm((3 * D, D), BF16),
        pltpu.SemaphoreType.DMA((9,)), pltpu.SemaphoreType.DMA((27,)),
    ]
    any_spec = pl.BlockSpec(memory_space=pl.ANY)
    outT, dxT, dwqkv, dwphi, dwo, dwg, dwu, dwdT = pl.pallas_call(
        _kernel,
        out_shape=out_shape,
        in_specs=[any_spec] * 8,
        out_specs=[any_spec] * 8,
        scratch_shapes=scratch,
        compiler_params=pltpu.CompilerParams(vmem_limit_bytes=126 * 1024 * 1024),
    )(xT, dyT, A_wqkv, wphi, A_wo, B_w_gate, B_w_up, wdT)

    return (outT.T.reshape(1, S, D), dxT.T.reshape(1, S, D), dwqkv,
            dwphi.reshape(DH, H, DH).transpose(1, 0, 2), dwo, dwg, dwu, dwdT.T)
```

```python
import jax
import jax.numpy as jnp
import jax.experimental.pallas as pl
import jax.experimental.pallas.tpu as pltpu

F32 = jnp.float32
BF16 = jnp.bfloat16
U32 = jnp.uint32

S, D, H, DH, DF = 2048, 448, 16, 28, 1792
NG = H // 2
GR = 2 * DH
GE = 64
GF = 2 * GR
T = 512
TH = T // 2
NT_ = S // T
NP = S // 2
DA, DB = 256, 192
DM = D // 2
MB = 512
NM = NP // MB
CH = ((0, 256), (512, 256), (1024, 256), (1536, 128))
LN_EPS = 1e-5
DEN_EPS = 1e-6
GELU_C1 = 0.7978845608028654
GELU_C2 = GELU_C1 * 0.044715
LOG2E = 1.4426950408889634


def _nn(a, b):
    return jnp.dot(a, b, preferred_element_type=F32)


def _nt(a, b):
    return jax.lax.dot_general(a, b, (((1,), (1,)), ((), ())),
                               preferred_element_type=F32)


def _iota(shape, dim):
    return jax.lax.broadcasted_iota(jnp.int32, shape, dim)


def _rows(*parts):
    return jnp.concatenate(parts, axis=0)


def _lanes(*parts):
    return jnp.concatenate(parts, axis=1)


def _seg_reduce(p, op, red, fill):
    low = _iota((p.shape[0], 8, p.shape[2]), 1) < 4
    v = [p[:, 8 * i:8 * i + 8, :] for i in range(7)]
    a = op(op(v[0], v[1]), op(v[2], jnp.where(low, v[3], fill)))
    b = op(op(v[4], v[5]), op(v[6], jnp.where(low, fill, v[3])))
    return red(a, axis=1, keepdims=True), red(b, axis=1, keepdims=True)


def _seg_mix(ra, rb):
    low = _iota((ra.shape[0], 8, ra.shape[2]), 1) < 4
    return jnp.where(low, ra, rb)


def _seg_sum(p):
    return _seg_reduce(p, jnp.add, jnp.sum, 0.0)


def _recip(x):
    r = pl.reciprocal(x, approx=True)
    return r * (2.0 - x * r)


def _pair_reduce(p, op):
    r = op(op(op(p[:, 0], p[:, 1]), op(p[:, 2], p[:, 3])), op(op(p[:, 4], p[:, 5]), p[:, 6]))
    r = op(r, pltpu.roll(r, 2, 1))
    r = op(r, pltpu.roll(r, 4, 1))
    return r[:, None]


def _softmax_pair(p):
    ep = jnp.exp2(p - _pair_reduce(p, jnp.maximum))
    en = jnp.exp2(_pair_reduce(p, jnp.minimum) - p)
    return ep * _recip(_pair_reduce(ep, jnp.add)), en * _recip(_pair_reduce(en, jnp.add))


def _softmax_pair_bwd(sp, sn, dsp, dsn):
    tp = sp * dsp
    tn = sn * dsn
    return (tp - sp * _pair_reduce(tp, jnp.add)) - (tn - sn * _pair_reduce(tn, jnp.add))


def _head_blocks(acc):
    r = _iota((NG, GE, GF), 1)
    c = _iota((NG, GE, GF), 2)
    row_b = ((r >= DH) & (r < GR)) | (r >= GR + 4)
    col_b = (c & 1) == 1
    m = jnp.where(row_b == col_b, acc, 0.0)
    padded = jnp.concatenate([m, jnp.zeros((NG, GE, 128 - GF), F32)], axis=2)
    z = padded.reshape(NG * GE, 128).T
    lane_lo = _iota((GF, 128), 1) < GE
    pairs = []
    for p in range(NG // 2):
        zp = z[:GF, 128 * p:128 * p + 128]
        pairs.append(jnp.concatenate(
            [jnp.where(lane_lo, zp, 0.0), jnp.where(lane_lo, 0.0, zp)], axis=0))
    return m.astype(BF16), jnp.stack(pairs).astype(BF16)


def _ffn_elem(g, u, dh):
    w = (GELU_C2 * g) * g
    t = jnp.tanh(g * (GELU_C1 + w))
    a = 0.5 + 0.5 * t
    ge = g * a
    gp = a + ge * (1.0 - a) * (2.0 * GELU_C1 + 6.0 * w)
    return ge * u, (u * gp) * dh, dh * ge


def _tie(x, t):
    if x.dtype == BF16:
        return pltpu.bitcast(_tie(pltpu.bitcast(x, U32), pltpu.bitcast(t, U32)), BF16)
    return jnp.where((_iota(x.shape, x.ndim - 1) >> 12) != 0, t, x)


def _all_rows(r):
    r = r + pltpu.roll(r, 4, 0)
    r = r + pltpu.roll(r, 2, 0)
    return r + pltpu.roll(r, 1, 0)


def _sum8(x):
    return jnp.sum(x.reshape(x.shape[0] // 8, 8, x.shape[1]), axis=0)


_XS = (3, 4, 6)
_YS = (2, 4, 5)


def _zext(b, like, axis):
    n = like.shape[axis] - b.shape[axis]
    if n == 0:
        return b
    shape = (n, b.shape[1]) if axis == 0 else (b.shape[0], n)
    return jnp.concatenate([b, jnp.zeros(shape, b.dtype)], axis=axis)


def _head(op, a, b):
    n = b.shape[0]
    return op(a, b) if n == a.shape[0] else _rows(op(a[:n], b), a[n:])


def _bf(ops):
    return [o.astype(BF16) for o in ops]


def _x_ops(x, k):
    lo, hi = [_lanes(x[:, h:h + TH], x[:, T + h:T + h + TH]) for h in (0, TH)]
    x11, x12, x21, x22 = lo[:k], lo[k:], hi[:k], hi[k:]
    return [_head(jnp.add, x11, x22), _head(jnp.add, x21, x22), x11, x22,
            x11[:D - k] + x12, x21 - x11, x12 - x22]


def _w_ops(lo, hi, k):
    kh = hi.shape[1]
    w11, w12, w21, w22 = lo[:k], hi[:k], lo[k:], hi[k:]
    w22e = _zext(w22, w21, 1)
    return [_head(jnp.add, w11, w22e), w11, _head(jnp.subtract, w12, w22),
            w21 - w11[:D - k], w22, w11[:, :kh] + w12, w21 + w22e]


def _wt_ops(a):
    f = a.shape[0] // 2
    w11, w21, w12, w22 = a[:f, :DA], a[:f, DA:], a[f:, :DA], a[f:, DA:]
    w22e = _zext(w22, w11, 1)
    return [w11 + w22e, w11, w12 - w22e, w21 - w11[:, :DB], w22, w11 + w12, w21 + w22]


def _y_ops(y11, y12, y21, y22):
    return _bf([y11 + y22, y21 - y22, y12 + y22, y11 + y21, y12 - y11, y22, y11])


def _yt_ops(y11, y12, y21, y22):
    n = y12.shape[0]
    return _bf([_head(jnp.add, y11, y22), _head(jnp.subtract, y21, y22), y12 + y22,
                y11 + y21, y12 - y11[:n], y22, y11])


def _y_blocks(p, p1, p4):
    return p[0] - p4 + p[3] + p[6], p4 + p[2], p1 + p[3], p[0] - p1 + p[2] + p[5]


def _y_now(p):
    return p[6] + p[0] + p[3] - p[4], p[4] + p[2], p[3] + p[1], p[5] + p[0] - p[1] + p[2]


def _x_half(h, p, tick):
    if h == 0:
        q = _tie(p[4], tick)
        return _rows(q + p[2] + p[0] - p[5], q + p[6])
    q = _tie(p[1], tick)
    return _rows(q + p[5], q + p[0] + p[3] - p[6])


def _w_from(p):
    return (p[1] + p[0] - p[3] + p[5], p[5] + p[2], p[6] + p[3],
            p[4] + p[0] - p[2] + p[6])


def _tri_left(a):
    return [a[0:128], _rows(a[128:192], a[64:128]), _rows(a[0:64], a[128:192])]


def _tri_right(b):
    b1, b2 = b[:, :128], b[:, 128:]
    return [_rows(b1[0:64], b2[64:128]),
            _rows(b1[128:192], b1[64:128] - b2[64:128]),
            _rows(b2[0:64] - b1[0:64], b2[128:192])]


def _tri_rows(a):
    r = a.shape[0] // 2
    a1, a2 = a[:r], a[r:]
    d = a1[:, :128] - a2[:, :128]
    first = _iota((r, 128), 1) < 64
    return [jnp.where(first, a1[:, :128], a2[:, :128]),
            _lanes(a1[:, 128:], d[:, 64:]),
            _lanes(-d[:, :64], a2[:, 128:])]


_TRI_K = ((0, 64), (128, 64), (0, 128))

GU = ("g", "u")
PQ, PV, PX = 208, 224, 32
PK = 2 * PQ + PV
PL = PK + 2 * PX
_P_OFF = (0, PQ, 2 * PQ)

_CHAIN = [g + s for g in (14, 0, 16, 2, 18, 4, 20, 6, 22, 8, 24, 10, 26, 12) for s in (0, 1)]
_PART = [_CHAIN.index(g) // 2 for g in range(28)]

RATE = 0.92
LAT = 200
JLAT = 1500
SEND_LAG = 1500
T_FFN = 231000
T_ATT = 235000
T_FIN = 265000
T_FILL = 185000


class _Task:
    def __init__(self, name, d, deps, fn, n=0, ops=0, lat=LAT, fence=False, rows=8):
        self.name, self.d, self.deps, self.fn = name, d, deps, fn
        self.n, self.v, self.lat, self.fence = n, ops / RATE, max(lat, JLAT) if n else lat, fence
        self.due, self.rel, self.rows = 0, [], rows


class _Plan:
    def __init__(self):
        self.mx, self.cnt, self.cols, self.later = [0] * 4, 0, [], []

    def note(self, p, k):
        m, n = p.shape
        for j in range(0, n, 128):
            st = 0
            for _ in range(0, k, 128):
                u = self.cnt % 4
                st = max(st, self.mx[u])
                self.mx[u] += m
                self.cnt += 1
            if j + 128 <= n:
                self.cols.append((st, m, p, j))
        return p

    def tick(self, r, rows):
        best = None
        for st, m, p, j in reversed(self.cols):
            row = min(max(-int((st - r) // 8) * 8, 0), m - rows)
            key = (st + row < r, abs(st + row - r))
            if best is None or key < best[0]:
                best = (key, p, row, j)
            if st + 4000 < r:
                break
        _, p, row, j = best
        return p[row:row + rows, j:j + 128]

    def run(self, tasks):
        pend = sorted([x for x in tasks if not x.n], key=lambda x: x.due)
        jobs = sorted([x for x in tasks if x.n], key=lambda x: x.due)
        done, vq = {}, 0.0
        when = lambda x: max([done.get(d, 1e18) for d in x.deps], default=0)

        def finish(x, t):
            done[x.name], done["order", x.name] = t + x.lat, 0

        while pend or jobs:
            t = min(self.mx)
            while self.later and self.later[0][0] <= t:
                self.later.pop(0)[1].start()
            ready = [x for x in pend if when(x) <= t]
            hold = bool(ready) and ready[0].fence
            while vq < t:
                cand = [x for x in jobs if when(x) <= t and (x.rel or not hold)]
                if not cand:
                    break
                vq = max(vq, min(when(x) for x in cand))
                x = [x for x in cand if when(x) <= vq][0]
                x.rel.append(vq)
                vq += x.v
                if len(x.rel) == x.n:
                    jobs.remove(x)
                    x.fn([self.tick(r, x.rows) for r in x.rel])
                    finish(x, vq)
            if hold and any(x.rel for x in jobs):
                ready = [x for x in ready if not x.fence]
            if not ready:
                self.mx = [max(u, t + 64) for u in self.mx]
                continue
            x = ready[0]
            pend.remove(x)
            x.fn()
            if x.fence:
                self.mx = [max(self.mx)] * 4
                self.cols = self.cols[-1:]
                vq = max(vq, self.mx[0])
            finish(x, max(self.mx) if x.d else t)
        for _, cp in self.later:
            cp.start()


def _kernel(xT_h, dyT_h, wqkv_h, wphi_h, wo_h, wg_h, wu_h, wdT_h,
            outT_h, dxT_h, dwqkv_h, dwphi_h, dwo_h, dwg_h, dwu_h, dwdT_h,
            xT, dyT, wqkv, wphi, wo, wg, wu, wdT,
            xnT, yo_s, phi_s, vext_s, yp_s, wqkvT,
            sem_in, sem_out):
    outT, dxT, dwqkv, dwphi, dwo, dwg, dwu, dwdT = xT, dyT, wqkv, wphi, wo, wg, wu, wdT
    cols = lambda i: slice(i * T, (i + 1) * T)
    prs = lambda i: slice(i * TH, (i + 1) * TH)
    blk = lambda m: slice(m * MB, (m + 1) * MB)
    two = lambda m: slice(2 * m * T, 2 * (m + 1) * T)

    in_list = [
        ("wphi", wphi_h, wphi),
        ("wo", wo_h, wo),
        ("dy0", dyT_h.at[:, cols(0)], dyT.at[:, cols(0)]),
        ("dy1", dyT_h.at[:, T:3 * T], dyT.at[:, T:3 * T]),
        ("dy2", dyT_h.at[:, cols(3)], dyT.at[:, cols(3)]),
        ("wd0", wdT_h.at[:, :2 * T], wdT.at[:, :2 * T]),
        ("x", xT_h, xT),
        ("wd1", wdT_h.at[:, 2 * T:], wdT.at[:, 2 * T:]),
        ("wqkv", wqkv_h, wqkv),
        ("wg", wg_h, wg),
        ("wu", wu_h, wu),
    ]
    in_cp = {}
    for n, (name, h, v) in enumerate(in_list):
        in_cp[name] = pltpu.make_async_copy(h, v, sem_in.at[n])
        in_cp[name].start()
    out_cp = []

    def send(src, dst):
        cp = pltpu.make_async_copy(src, dst, sem_out.at[len(out_cp)])
        plan.later.append((min(plan.mx) + SEND_LAG, cp))
        out_cp.append(cp)

    V = {}
    plan = _Plan()

    def nn(a, b):
        return plan.note(_nn(a, b), a.shape[1])

    def nt(a, b):
        return plan.note(_nt(a, b), a.shape[1])

    def strip(tk):
        return _lanes(tk[0], tk[1], tk[0], tk[1], tk[2], tk[3], tk[2], tk[3])

    def acc(key, val):
        V[key] = val + V[key] if key in V else val

    def wait(*names):
        for n in names:
            in_cp[n].wait()

    def tri(lhs, rhs):
        e = nn(lhs(0), rhs(0))
        c1 = nn(lhs(1), rhs(1)) + e
        return c1, nn(lhs(2), rhs(2)) + e

    def tri_rhs(ref, idx, r0, lanes):
        return lambda k: _rows(*[ref[(*idx, slice(r0 + o, r0 + o + 64), lanes)] for o in _TRI_K[k]])

    def prep_x(which, m, x):
        ops = _x_ops(x, DA)
        q4 = range(0, MB, 128)
        pcs = [_bf(_tri_left(op) if n in _XS else [op[:128], op[128:]]) for n, op in enumerate(ops)]
        V["xb", which, m] = [
            _bf([op]) if n not in _XS else pcs[n] if which else
            [_bf(_tri_left(op[:, l:l + 128])) for l in q4] for n, op in enumerate(ops)]
        xf = [[pc.T for pc in q] for q in pcs]
        V["xf", which, m] = [[[pc[l:l + 128] for pc in q] for l in q4] if n in _XS else [q]
                             for n, q in enumerate(xf)]
        V["xw", which, m] = _bf(_x_ops(x, DM))

    def prep_dy(m, tk):
        st = [strip(tk[k::14]) for k in range(14)]
        prep_x(1, m, _tie(dyT[:, two(m)], _rows(*[st[k] for k in _PART])).astype(F32))

    def prep_w(group, c):
        c0, w = CH[c]
        fw, rw = [], []
        for ref in {"d": (wdT,), "gu": (wg, wu)}[group]:
            lo = ref[:, c0:c0 + w].astype(F32)
            hi = ref[:, c0 + w:c0 + 2 * w].astype(F32)
            fw.append([[op[:128], op[128:]] if n not in _XS else _tri_right(op) if w == 256 else
                       [op[:128], _rows(op[128:], jnp.zeros((64, w), F32))]
                       for n, op in enumerate(_w_ops(lo, hi, DA))])
            rw.append(_w_ops(lo, hi, DM))
        if w == 128:
            fw = [[[_lanes(*pc) for pc in zip(*[f[n] for f in fw])] for n in range(7)]]
        for nm, f in zip(group, fw):
            V["wf", nm, c] = [_bf(ops) for ops in f]
        V["wr", group, c] = _bf([_lanes(*ops) for ops in zip(*rw)])

    def prep_t(name, a):
        V["wt", name] = [_bf(_tri_rows(op) if n in _XS else [op])
                         for n, op in enumerate(_wt_ops(a))]

    def f_mm(names, c, m, n):
        which, w = int(names[0] == "d"), CH[c][1]
        lhs, rhs = V["xf", which, m][n], V["wf", names[0], c][n]
        if len(rhs) == 3:
            p = _rows(*[_lanes(*tri(lambda k: q[k], lambda k: rhs[k])) for q in lhs])
        else:
            p = _rows(*[nn(q[0], rhs[0]) + nn(q[1], rhs[1]) for q in lhs])
        for k, nm in enumerate(names):
            V["p", nm, c, m, n] = p[:, k * w:(k + 1) * w]
        if which and n == 6:
            V["dh", c, m] = _y_now([V.pop(("p", "d", c, m, k)) for k in range(7)])

    def t_f(group, c, m, extra):
        w, which = CH[c][1], int(group == "d")
        deps = [("pw", group, c), ("px", which, m)] + extra
        out = []
        for names in ([("g",), ("u",)] if group == "gu" and w == 256 else [tuple(group)]):
            for n in range(7):
                d = MB * len(names) // 2 if w == 128 else (384 if n in _XS else MB)
                out.append(_Task(("f", names[-1], c, m, n), d, deps,
                                 lambda n=n, names=names: f_mm(names, c, m, n)))
                deps = [("order", out[-1].name)]
        return out

    def gelu(c, m, tk):
        nl = CH[c][1] // 128
        ta = _rows(*[r for k in range(0, len(tk), nl) for r in [_lanes(*tk[k:k + nl])] * 2])
        ys = []
        for nm in GU:
            p = [V.pop(("p", nm, c, m, n)) for n in range(7)]
            ys.append(_y_blocks(p, _tie(p[1], ta), _tie(p[4], ta)))
        e = {b: _ffn_elem(ys[0][b], ys[1][b], V["dh", c, m][b]) for b in (2, 3, 1, 0)}
        del V["dh", c, m]
        h, dg, du = zip(*[e[b] for b in range(4)])
        V["z", 1, c, m] = _y_ops(*h)
        V["z", 0, c, m] = _y_ops(*[_lanes(a, b) for a, b in zip(dg, du)])

    def acc_x(which, m, n, val, l0=0):
        for l in range(0, val.shape[1], 128):
            acc(("ax", which, m, n, (l0 + l) // 128), val[:, l:l + 128])

    def bwd_x(which, c, m, n):
        lhs = V["wr", "d" if which else "gu", c][n]
        acc_x(which, m, n, nt(lhs, V["z", which, c, m][n]))

    def bwd_w(which, c, m, n):
        acc(("aw", which, c, n), nn(V["xw", which, m][n], V["z", which, c, m][n]))

    def fin_w(which, c):
        c0, w = CH[c]
        q = _w_from([V.pop(("aw", which, c, n)) for n in range(7)])
        refs = ((dwg, dwg_h), (dwu, dwu_h)) if which == 0 else ((dwdT, dwdT_h),)
        for k, (ref, hbm) in enumerate(refs):
            sl = slice(k * w, (k + 1) * w)
            ref[:DM, c0:c0 + w] = q[0][:, sl].astype(BF16)
            ref[:DM, c0 + w:c0 + 2 * w] = q[1][:, sl].astype(BF16)
            ref[DM:, c0:c0 + w] = q[2][:, sl].astype(BF16)
            ref[DM:, c0 + w:c0 + 2 * w] = q[3][:, sl].astype(BF16)
            if which and c == len(CH) - 1:
                for l in (c0, c0 + w):
                    send(ref.at[:, l:l + w], hbm.at[:, l:l + w])
            else:
                send(ref.at[:, c0:c0 + 2 * w], hbm.at[:, c0:c0 + 2 * w])

    W_ORD = (0, 2, 3, 5, 6, 1, 4)
    X_ORD = (1, 3, 0, 6, 5, 2, 4)

    def t_bx(c, m):
        d = DM * CH[c][1] // 128
        return [_Task(("bx", which, c, m, n), d * (2 - which), [("ge", c, m)],
                      lambda which=which, n=n: bwd_x(which, c, m, n))
                for which in (1, 0) for n in X_ORD]

    def t_bw(which, c, m):
        d = DM * CH[c][1] // 128 * (2 - which)
        out = []
        for n in W_ORD:
            deps = [("ge", c, m)] + ([("order", ("bw", which, c, m - 1, n))] if m else [])
            out.append(_Task(("bw", which, c, m, n), d, deps,
                             lambda n=n: bwd_w(which, c, m, n)))
        if m == NM - 1:
            out.append(_Task(("fw", which, c), 0, [("order", t.name) for t in out],
                             lambda: fin_w(which, c)))
        return out

    def consts():
        r = _iota((D, D), 0)
        c = _iota((D, D), 1)
        V["perm"] = jnp.where(r == (c & 15) * DH + (c >> 4), 1.0, 0.0).astype(BF16)
        V["perm_t"] = jnp.where(c == (r & 15) * DH + (r >> 4), 1.0, 0.0).astype(BF16)
        rr = _iota((GF, DH), 0)
        rc = _iota((GF, DH), 1)
        V["rep"] = jnp.where((rr >> 1 == rc) | (rr >> 1 == rc + DH), 1.0, 0.0).astype(BF16)
        br = _iota((GF, GF), 0)
        bc = _iota((GF, GF), 1)
        hd = lambda t: ((t >= DH).astype(jnp.int32) + (t >= 2 * DH).astype(jnp.int32)
                        + (t >= 3 * DH).astype(jnp.int32))
        hf = lambda t: 2 * (t >= GR).astype(jnp.int32) + (t & 1)
        V["diag_t"] = jnp.where(hf(br) == hd(bc), 1.0, 0.0)
        V["diag"] = jnp.where(hd(br) == hf(bc), 1.0, 0.0)

    def phi_a():
        V["wphi_hd"] = nn(V["perm"], wphi[...]).astype(BF16)

    def phi_b():
        whd, rep, diag = V["wphi_hd"], V["rep"], V["diag"] > 0.5
        V["phi_t"] = [jnp.where(V["diag_t"] > 0.5, nt(rep, whd[GF * g:GF * g + GF]), 0.0).astype(BF16)
                      for g in range(4)]
        V["phi_n"] = [jnp.where(diag, nt(whd[GF * g:GF * g + GF], rep), 0.0).astype(BF16)
                      for g in range(4)]

    def prep_wo():
        woT = wo[...].T.astype(F32)
        V["wa"] = [_bf(_tri_rows(op) if n in _YS else [op])
                   for n, op in enumerate(_w_ops(woT[:, :DA], woT[:, DA:], DM))]

    def tr_qkv():
        wqkvT[...] = wqkv[...].T

    def fold(t):
        if t < 2:
            V["WT", t] = _rows(*[nn(V["phi_t"][g], wqkvT[D * t + GF * g:D * t + GF * g + GF, :])
                                 for g in range(4)])
        else:
            V["WT", t] = wqkvT[2 * D:, :].astype(F32)
        prep_t(t, V["WT", t] * LOG2E if t < 2 else V["WT", t])

    def prep_wp():
        q, k, v = [V.pop(("WT", t)) for t in range(3)]
        lo = _rows(q[:PQ], k[:PQ], v[:PV], q[2 * PQ:], k[2 * PQ:]).T
        hi = _rows(q[PQ:2 * PQ], k[PQ:2 * PQ], v[PV:]).T
        V["wp"] = [_bf([op] if n in _YS else [op[:, :PL - DB]] + _tri_rows(op[:, PL - DB:]))
                   for n, op in enumerate(_w_ops(lo, hi, DM))]

    def ln(m, tk):
        xb = xT[:, two(m)]
        x0 = jnp.broadcast_to(xT[:16, two(m)].astype(F32)[:1], (8, 2 * T))
        ta = [_lanes(*tk[s:56:7]) for s in range(7)]
        xs = _tie(xb, _rows(*[ta[g // 4] for g in range(28)])).astype(F32) - _rows(*[x0] * (D // 8))
        s1, s2 = [_all_rows(_sum8(_rows(*[_sum8(v[r:r + 64]) for r in range(0, D, 64)]))) * (1.0 / D)
                  for v in (xs, xs * xs)]
        rstd = jax.lax.rsqrt(s2 - s1 * s1 + LN_EPS)
        V["rstd", m] = rstd
        tc = [strip(tk[56 + 3 * k // 2::21]) for k in range(14)]
        x = _tie(xb, _rows(*[tc[k] for k in _PART])).astype(F32)
        xn = (x - _rows(*[x0 + s1] * (D // 8))) * _rows(*[rstd] * (D // 8))
        xnT[:, two(m)] = xn.astype(BF16)
        prep_x(0, m, xn)

    def a_sink(t, m, ys):
        for b, y in enumerate(ys):
            h, f = divmod(b, 2)
            gs = slice(4 * f, 4 * f + 4)
            if t == 2:
                y = jnp.concatenate([y.reshape(4, GR, MB), jnp.ones((4, 8, MB), F32)],
                                    axis=1).astype(BF16)
            else:
                y = jnp.concatenate(_softmax_pair(y.reshape(4, 7, 8, MB)),
                                    axis=1).reshape(4, GF, MB).astype(BF16)
            for s in range(2):
                c0 = (2 * m + s) * T + h * TH
                part = y[..., s * TH:s * TH + TH]
                if t == 2:
                    vext_s[gs, :, c0:c0 + TH] = part
                else:
                    phi_s[t, gs, :, c0:c0 + TH] = part

    def a_mm(t, m, n):
        lhs, rhs = V["wt", t][n], V["xb", 0, m][n]
        V["ap", t, m, n] = (_lanes(*[_rows(*tri(lambda s: lhs[s], lambda s: q[s])) for q in rhs])
                            if n in _XS else nn(lhs[0], rhs[0]))
        if n == 6 and t == 2:
            a_sink(t, m, _y_now([V.pop(("ap", t, m, k)) for k in range(7)]))

    def feat(t, m, tk):
        p = [V.pop(("ap", t, m, k)) for k in range(7)]
        ta = [_rows(*[_lanes(*tk[4 * g + s::16]) for g in range(4)]) for s in range(4)]
        a_sink(t, m, (p[0] - _tie(p[4], ta[0]) + p[3] + p[6], _tie(p[4], ta[1]) + p[2],
                      _tie(p[1], ta[2]) + p[3], p[0] - _tie(p[1], ta[3]) + p[2] + p[5]))

    def t_proj(t, m):
        deps = [("pt", t), ("px", 0, m)]
        out = []
        for n in range(7):
            out.append(_Task(("ap", t, m, n), 3 * DM // 2 if n in _XS else 2 * DM, deps,
                             lambda n=n: a_mm(t, m, n)))
            deps = [("order", out[-1].name)]
        if t in (0, 1):
            out.append(_Task(("sm", t, m), 0, [out[-1].name], lambda tk: feat(t, m, tk), 64, 124,
                             rows=56))
        return out

    def do_plain(i):
        p = nn(wo[...], dyT[:, cols(i)])
        for f in range(2):
            for h in range(2):
                V["do", f, i * T + h * TH] = p[DM * f:DM * f + DM, h * TH:h * TH + TH]

    def k_state(i, p):
        for j in (2 * p, 2 * p + 1):
            acc(("kv", j), nt(vext_s[j, :, cols(i)], phi_s[1, j, :, cols(i)]))

    def blocks(name):
        V[name, "T"], V[name, "P"] = _head_blocks(jnp.stack([V.pop((name, j)) for j in range(NG)]))

    def ne_mm(i, p):
        for j in (2 * p, 2 * p + 1):
            V["ne", i, j] = nn(V["kv", "T"][j], phi_s[0, j, :, cols(i)])

    def q_mid(i, tk):
        low = _iota((NG, 8, T), 1) < 4
        ne = jnp.stack([V.pop(("ne", i, j)) for j in range(NG)])
        pos = (1, 3, 5, 7, 0, 2, 4, 6)
        rmix = _recip(_tie(ne[:, GR:, :], jnp.stack(
            [_lanes(*[tk[4 * k + l] for l in (0, 2, 1, 3)]) for k in pos]))
                      + DEN_EPS)
        rrot = pltpu.roll(rmix, 4, 1)
        ra = jnp.where(low, rmix, rrot)
        rb = jnp.where(low, rrot, rmix)
        rden = jnp.concatenate([ra, ra, ra, rmix, rb, rb, rb], axis=1)
        o = ne[:, :GR, :] * rden
        do = _rows(*[_lanes(*[V.pop(("do", f, i * T + l)) for l in (0, TH)]) for f in range(2)])
        dnum = do.reshape(NG, GR, T) * rden
        dden = _seg_mix(*_seg_sum(dnum * o)) * (-0.25)
        V["dne", i] = jnp.concatenate([dnum, dden], axis=1).astype(BF16)
        o = o.reshape(D, T)
        for n, op in enumerate(_yt_ops(o[:DA, :TH], o[DA:, :TH], o[:DA, TH:], o[DA:, TH:])):
            yo_s[n, :op.shape[0], prs(i)] = op

    def dp_put(t, i, y):
        r, off = (PV if t == 2 else PQ), _P_OFF[t]
        for n, op in enumerate(_y_ops(y[:r, :TH], y[r:2 * r, :TH], y[:r, TH:], y[r:2 * r, TH:])):
            yp_s[n, off:off + r, prs(i)] = op
        if t < 2:
            lo, hi = y[2 * r:, :TH], y[2 * r:, TH:]
            for n, op in zip((0, 1, 3, 6), _bf([lo, hi, lo + hi, lo])):
                yp_s[n, PK + PX * t:PK + PX * t + PX, prs(i)] = op

    def dphi_mm(t, i, p):
        if t == 0:
            rhs = V["dne", i][2 * p:2 * p + 2]
        else:
            rhs = vext_s[2 * p:2 * p + 2, :, cols(i)]
        V["dphi", t, i, p] = nn(V["dkv" if t else "kv", "P"][p], rhs.reshape(2 * GE, T))

    def phi_bwd(t, i, tk):
        dphi = _rows(*[V.pop(("dphi", t, i, p)) for p in range(4)]).reshape(NG, 14, 8, T)
        pos = (0, 2, 4, 6, 1, 3, 5, 7)
        ta = _rows(*[_lanes(*[tk[4 * k + l] for l in (0, 2, 1, 3)]) for k in pos])
        pf = _tie(phi_s[t, :, :, cols(i)].reshape(NG * GF, T), ta)
        pf = pf.astype(F32).reshape(NG, 14, 8, T)
        dp = _softmax_pair_bwd(pf[:, :7], pf[:, 7:], dphi[:, :7], dphi[:, 7:])
        dp_put(t, i, dp.reshape(D, T))

    def q_state(i, p):
        for j in (2 * p, 2 * p + 1):
            acc(("dkv", j), nt(V["dne", i][j], phi_s[0, j, :, cols(i)]))

    def dv_mm(i, p):
        for j in (p, p + 4):
            V["dv", i, j] = nn(V["dkv", "T"][j], phi_s[1, j, :, cols(i)])[:GR]
        if p == 3:
            dp_put(2, i, _rows(*[V.pop(("dv", i, j)) for j in range(NG)]))

    def x_tri(name, which, wname, ref, r0, m, n, deps):
        def run():
            for l in range(0, MB, 128):
                acc_x(which, m, n, _rows(*tri(
                    lambda s: V[wname][n][s - 3],
                    tri_rhs(ref, (n,), r0, slice(m * MB + l, m * MB + l + 128)))), l)
        return _Task(name, 3 * DM // 2, deps, run)

    def t_outa(m):
        deps = [("qm", 2 * m), ("qm", 2 * m + 1), "pwo"]
        return [x_tri(("oa", m, n), 1, "wa", yo_s, 0, m, n, deps) if n in _YS else
                _Task(("oa", m, n), 2 * DM, deps,
                      lambda n=n: acc_x(1, m, n, nn(V["wa"][n][0], yo_s[n, :, blk(m)])))
                for n in X_ORD]

    def dwo_mm(m, n):
        lhs, rhs = yo_s[n, :DB if n in _YS else DA, blk(m)], V["xb", 1, m][n]
        p = nt(lhs, rhs[0])
        acc(("ao", n), _lanes(p, nt(lhs, rhs[1])[:, :64]) if n in _XS else p)

    def fin_wo():
        p = [V.pop(("ao", n)) for n in range(7)]
        dwo[:DA, :DA] = _head(jnp.add, p[1] + p[0] - _zext(p[3], p[0], 1), p[5]).astype(BF16)
        dwo[DA:, :DA] = (p[5] + p[2]).astype(BF16)
        dwo[:DA, DA:] = (p[6] + p[3]).astype(BF16)
        dwo[DA:, DA:] = (p[4] + p[0][:DB, :DB] - p[2][:, :DB] + p[6][:DB]).astype(BF16)
        send(dwo, dwo_h)

    def t_dwo(m):
        out = [_Task(("ao", m, n), 2 * (DB if n in _YS else DA),
                     [("qm", 2 * m), ("qm", 2 * m + 1)]
                     + ([("order", ("ao", m - 1, n))] if m else []),
                     lambda n=n: dwo_mm(m, n)) for n in W_ORD]
        if m == NM - 1:
            out.append(_Task("fwo", 0, [("order", t.name) for t in out], fin_wo))
        return out

    def dp_deps(m):
        return [d for i in (2 * m, 2 * m + 1) for d in (("pb", 0, i), ("pb", 1, i), ("dv", i, 3))]

    def t_dxn(m):
        out = []
        deps = dp_deps(m) + ["pwp"]
        for n in X_ORD:
            if n in _YS:
                out.append(_Task(("dx", m, n), 5 * DM, deps, lambda n=n: acc_x(
                    0, m, n, nn(V["wp"][n][0], yp_s[n, :PK, blk(m)]))))
            else:
                out.append(_Task(("dx", m, n, 0), 4 * DM, deps, lambda n=n: acc_x(
                    0, m, n, nn(V["wp"][n][0], yp_s[n, :PL - DB, blk(m)]))))
                out.append(x_tri(("dx", m, n), 0, "wp", yp_s, PL - DB, m, n,
                                 [("order", out[-1].name)]))
        return out

    def g_mm(m, n):
        acc(("ag", n), nt(V["xw", 0, m][n], yp_s[n, :PK, blk(m)]))

    def gx_mm(i):
        acc("gx", nt(_lanes(yp_s[0, PK:, prs(i)], yp_s[1, PK:, prs(i)]), xnT[:, cols(i)]))

    def t_g(m):
        out = [_Task(("gx", i), 4 * GE, dp_deps(m), lambda i=i: gx_mm(i))
               for i in (2 * m, 2 * m + 1)]
        out += [_Task(("ag", m, n), 5 * DM,
                      dp_deps(m) + ([("order", ("ag", m - 1, n))] if m else []),
                      lambda n=n: g_mm(m, n)) for n in W_ORD]
        return out

    need = ((4, 2, 0, 5, 6), (1, 5, 0, 3, 6))

    def x_prod(which, m, h):
        return {n: _lanes(*[V["ax", which, m, n, k] for k in range(4)]) for n in need[h]}

    def half_cols(ref, m, h):
        return [ref.at[:, i * T + h * TH:i * T + h * TH + TH] for i in (2 * m, 2 * m + 1)]

    def fin_out(m, h, tk):
        st = [_lanes(*tk[s::7]) for s in range(7)]
        ta = _rows(*[st[g // 4] for g in range(28)])
        tb = _rows(*[st[g % 14 // 2] for g in range(28)])
        x = _tie(_lanes(*[r[...] for r in half_cols(xT, m, h)]), tb).astype(F32)
        out = (_x_half(h, x_prod(1, m, h), ta) + x).astype(BF16)
        for s, (a, b) in enumerate(zip(half_cols(outT, m, h), half_cols(outT_h, m, h))):
            a[...] = out[:, s * TH:s * TH + TH]
            send(a, b)

    def fin_dx(m, h, tk):
        st = [_lanes(*tk[s:28:7]) for s in range(7)]
        sb = [_lanes(*tk[28 + s::7]) for s in range(7)]
        dxn = _x_half(h, x_prod(0, m, h), _rows(*[st[g // 4] for g in range(28)]))
        xf = _tie(_lanes(*[r[...] for r in half_cols(xnT, m, h)]),
                  _rows(*[st[g % 14 // 2] for g in range(28)])).astype(F32)
        m1, m2 = [_all_rows(_sum8(_rows(*[_sum8(v[r:r + 32] + v[DM + r:DM + r + 32])
                                          for r in range(0, DM, 32)]))) * (1.0 / D)
                  for v in (dxn, dxn * xf)]
        rstd = _lanes(*[V["rstd", m][:, l + h * TH:l + h * TH + TH] for l in (0, T)])
        m1, m2 = [_rows(*[r for s in sb for r in [_tie(v, s)] * 8]) for v in (m1, m2)]
        dy = _lanes(*[r[...] for r in half_cols(dyT, m, h)]).astype(F32)
        dx = ((dxn - m1 - xf * m2).reshape(D // 8, 8, MB) * rstd[None]).reshape(D, MB) + dy
        dx = dx.astype(BF16)
        for s, (a, b) in enumerate(zip(half_cols(dxT, m, h), half_cols(dxT_h, m, h))):
            a[...] = dx[:, s * TH:s * TH + TH]
            send(a, b)

    def unfold_a():
        w11, w12, w21, w22 = _w_from([V.pop(("ag", n)) for n in range(7)])
        lo = _rows(w11, w21).astype(BF16).T
        hi = _rows(w12, w22).astype(BF16).T
        gx = V.pop("gx").astype(BF16)
        V["gT"] = _rows(lo[:PQ], hi[:PQ], gx[:PX], lo[PQ:2 * PQ], hi[PQ:2 * PQ], gx[PX:],
                        lo[2 * PQ:], hi[2 * PQ:])

    def unfold_b():
        gT = V["gT"]
        dwT = _rows(*[nn(V["phi_n"][g % 4], gT[GF * g:GF * g + GF]).astype(BF16)
                      for g in range(8)], gT[2 * D:])
        dwqkv[...] = dwT.T
        send(dwqkv, dwqkv_h)

    def unfold_c():
        gT = V["gT"]
        diag = V["diag"] > 0.5
        V["xqk"] = []
        for g in range(4):
            xq = nt(wqkvT[GF * g:GF * g + GF, :], gT[GF * g:GF * g + GF])
            xk = nt(wqkvT[D + GF * g:D + GF * g + GF, :], gT[D + GF * g:D + GF * g + GF]) + xq
            V["xqk"].append(jnp.where(diag, xk, 0.0).astype(BF16))

    def unfold_d():
        V["ys"] = _rows(*[nn(t, V["rep"]).astype(BF16) for t in V.pop("xqk")])

    def unfold_e():
        dwphi[...] = nn(V["perm_t"], V.pop("ys")).astype(BF16)
        send(dwphi, dwphi_h)

    def spread(tasks, t0, t1):
        tot, pos = sum(x.d for x in tasks), 0
        for x in tasks:
            x.due = t0 + (t1 - t0) * pos / max(tot, 1)
            pos += x.d
        return tasks

    nc = len(CH)
    q4 = range(4)
    px_dy = lambda m: _Task(("px", 1, m), 0, ["w3" if m else "w2"],
                            lambda tk: prep_dy(m, tk), 56, 48)
    px_x = lambda m: _Task(("px", 0, m), 0, ["w4"], lambda tk: ln(m, tk), 140, 44)
    start = [
        px_dy(0), px_dy(1), px_x(0), px_x(1),
        _Task("w0", 0, [], lambda: wait("wphi"), lat=0, fence=True),
        _Task("phi_a", D, ["w0"], phi_a, lat=0),
        _Task("phi_b", 2 * GF, ["phi_a"], phi_b)]

    def fence(name, *names):
        start.append(_Task(name, 0, [("order", start[-1].name)], lambda: wait(*names),
                           lat=0, fence=True))

    def then(w, *tasks):
        for x in tasks:
            x.deps = x.deps + [w]
            start.append(x)

    t_do = lambda i: _Task(("do", i), 4 * D, [], lambda: do_plain(i))
    t_pw = lambda c: _Task(("pw", "d", c), 0, [], lambda: prep_w("d", c), lat=0)
    fence("w1", "wo", "dy0")
    then("w1", t_do(0))
    fence("w2", "dy1")
    then("w2", t_do(1), t_do(2))
    fence("w3", "dy2", "wd0")
    fd = {(c, m): t_f("d", c, m, []) for c in range(nc) for m in range(NM)}
    then("w3", t_pw(0), t_do(3), t_pw(1), *fd[0, 0], *fd[1, 0][:4])
    fence("w4", "x", "wd1")
    then("w4", *fd[1, 0][4:], *fd[0, 1], t_pw(2), *fd[1, 1], *fd[2, 0], t_pw(3), *fd[2, 1],
         *fd[3, 0][:2])
    fence("w5", "wqkv", "wg", "wu")
    then("w5", *fd[3, 0][2:])
    spread(start, 0, 30000)
    start += spread(fd[3, 1], T_FILL, T_FILL + 1)

    prep = [_Task("trq", 0, ["w5"], tr_qkv, lat=2000),
            _Task(("pt", 1), D, ["trq", "phi_b"], lambda: fold(1), lat=1000),
            _Task(("pt", 2), 0, ["trq"], lambda: fold(2), lat=1000),
            _Task(("pt", 0), D, ["trq", "phi_b"], lambda: fold(0), lat=1000),
            _Task("pwo", 0, ["w5"], prep_wo)]
    for x, due in zip(prep, (0, 0, 36000, 45000, 100000)):
        x.due = due

    steps = [(c, m) for c in range(nc) for m in range(NM)]

    def s_f(k):
        c, m = steps[k]
        out = [] if m else [_Task(("pw", "gu", c), 0, ["w5"], lambda: prep_w("gu", c), lat=0)]
        out += t_f("gu", c, m, [("ge", *steps[min(k - 2, 4)])] if k > 1 else [])
        return out + [_Task(("ge", c, m), 0, [("f", "u", c, m, 6), ("f", "d", c, m, 6)],
                            lambda tk: gelu(c, m, tk), CH[c][1] // 4, 220)]

    s_x = lambda k: t_bx(*steps[k])
    s_w = lambda k: t_bw(0, *steps[k]) + t_bw(1, *steps[k])
    ffn = s_f(0)
    for k in range(4):
        ffn += s_f(k + 1) + s_x(k) + s_w(k)
    ffn += s_f(5) + s_x(4) + s_f(6) + s_f(7) + s_w(4)
    late = s_w(5) + [x for w in (0, 1) for m in (0, 1) for x in t_bw(w, 3, m)]
    spread(ffn, 30000, T_FFN)

    att = []
    for m in range(NM):
        att += t_proj(1, m) + t_proj(2, m)
    for m in range(NM):
        att += [_Task(("ks", i, p), 2 * GE, [("sm", 1, m), ("ap", 2, m, 6)],
                      lambda i=i, p=p: k_state(i, p)) for i in (2 * m, 2 * m + 1) for p in q4]
        att += t_proj(0, m)
    att.append(_Task("kv", 0, [("ks", i, p) for i in q4 for p in q4], lambda: blocks("kv"),
                     lat=600))
    att.append(_Task("pwp", 0, [("pt", t) for t in range(3)], prep_wp))
    for m in range(NM):
        for i in (2 * m, 2 * m + 1):
            att += [_Task(("ne", i, p), 2 * GE, ["kv", ("sm", 0, m)], lambda i=i, p=p: ne_mm(i, p))
                    for p in q4]
            att.append(_Task(("qm", i), 0, [("ne", i, p) for p in q4],
                             lambda tk, i=i: q_mid(i, tk), 32, 95))
        for i in (2 * m, 2 * m + 1):
            att += [_Task(("qs", i, p), 2 * GE, [("qm", i)], lambda i=i, p=p: q_state(i, p))
                    for p in q4]
            att += [_Task(("dphi", 0, i, p), DM, [("qm", i)], lambda i=i, p=p: dphi_mm(0, i, p))
                    for p in q4]
            att.append(_Task(("pb", 0, i), 0, [("dphi", 0, i, p) for p in q4],
                             lambda tk, i=i: phi_bwd(0, i, tk), 32, 100, rows=56))
        att += t_outa(m) + t_dwo(m)
    att.append(_Task("dkv", 0, [("qs", i, p) for i in q4 for p in q4], lambda: blocks("dkv"),
                     lat=600))
    for m in range(NM):
        for i in (2 * m, 2 * m + 1):
            att += [_Task(("dphi", 1, i, p), DM, ["dkv"], lambda i=i, p=p: dphi_mm(1, i, p))
                    for p in q4]
            att.append(_Task(("pb", 1, i), 0, [("dphi", 1, i, p) for p in q4],
                             lambda tk, i=i: phi_bwd(1, i, tk), 32, 100, rows=56))
            att += [_Task(("dv", i, p), 2 * GE,
                          ["dkv"] + ([("order", ("dv", i, p - 1))] if p else []),
                          lambda i=i, p=p: dv_mm(i, p)) for p in q4]
    for m in range(NM):
        att += t_g(m)
    att += [_Task("ua", 0, [("ag", NM - 1, n) for n in range(7)] + [("gx", i) for i in q4],
                  unfold_a, lat=2500),
            _Task("ub", 8 * GF, ["ua"], unfold_b),
            _Task("uc", 8 * GF, ["ua"], unfold_c, lat=800),
            _Task("ud", GF, ["uc"], unfold_d, lat=800),
            _Task("ue", D, ["ud"], unfold_e)]
    spread(att, 31000, T_ATT)

    fin = []
    for m in range(NM):
        fin += s_x(5) + s_x(7) if m else s_x(6)
        for h in (1, 0):
            fin.append(_Task(("fo", m, h), 0,
                             [("bx", 1, c, m, n) for c in range(nc) for n in need[h]]
                             + [("oa", m, n) for n in need[h]],
                             lambda tk, m=m, h=h: fin_out(m, h, tk), 28, 60))
        fin += t_dxn(m)
        for h in (1, 0):
            fin.append(_Task(("fdx", m, h), 0,
                             [("bx", 0, c, m, n) for c in range(nc) for n in need[h]]
                             + [("dx", m, n) for n in need[h]],
                             lambda tk, m=m, h=h: fin_dx(m, h, tk), 56, 65))
    spread(fin, T_ATT, T_FIN)
    spread(late, T_FIN, T_FIN + 20000)

    consts()
    plan.run(start + prep + ffn + att + fin + late)
    for cp in out_cp:
        cp.wait()


@jax.jit
def pallas_parallel_sum__linear_kernel_hedgehog__glu_gated_geglu__prompt_kernel(
    A_x: jax.Array,
    A_wqkv: jax.Array,
    A_w_phi: jax.Array,
    A_wo: jax.Array,
    B_x: jax.Array,
    B_w_gate: jax.Array,
    B_w_up: jax.Array,
    B_w_down: jax.Array,
    grad_out: jax.Array,
):
    del B_x
    xT = A_x.reshape(S, D).T
    dyT = grad_out.reshape(S, D).T
    wphi = A_w_phi.transpose(1, 0, 2).reshape(DH * H, DH)
    wdT = B_w_down.T

    vm = pltpu.VMEM
    sds = lambda *s: jax.ShapeDtypeStruct(s, BF16)
    out_shape = (sds(D, S), sds(D, S), sds(D, 3 * D), sds(D, DH), sds(D, D),
                 sds(D, DF), sds(D, DF), sds(D, DF))
    scratch = [
        vm((D, S), BF16), vm((D, S), BF16), vm((D, 3 * D), BF16), vm((D, DH), BF16),
        vm((D, D), BF16), vm((D, DF), BF16), vm((D, DF), BF16), vm((D, DF), BF16),
        vm((D, S), BF16), vm((7, DA, NP), BF16),
        vm((2, NG, GF, S), BF16), vm((NG, GE, S), BF16),
        vm((7, PL, NP), BF16), vm((3 * D, D), BF16),
        pltpu.SemaphoreType.DMA((11,)), pltpu.SemaphoreType.DMA((32,)),
    ]
    any_spec = pl.BlockSpec(memory_space=pl.ANY)
    outT, dxT, dwqkv, dwphi, dwo, dwg, dwu, dwdT = pl.pallas_call(
        _kernel,
        out_shape=out_shape,
        in_specs=[any_spec] * 8,
        out_specs=[any_spec] * 8,
        scratch_shapes=scratch,
        compiler_params=pltpu.CompilerParams(vmem_limit_bytes=126 * 1024 * 1024),
    )(xT, dyT, A_wqkv, wphi, A_wo, B_w_gate, B_w_up, wdT)

    return (outT.T.reshape(1, S, D), dxT.T.reshape(1, S, D), dwqkv,
            dwphi.reshape(DH, H, DH).transpose(1, 0, 2), dwo, dwg, dwu, dwdT.T)
```
